```python
import os as _os
_os.environ.setdefault("JAX_PLATFORMS", "cpu")
import jax
import jax.numpy as jnp

def _softmax(x, axis=-1):
    return jax.nn.softmax(x, axis=axis)
def _gelu(x):
    return jax.nn.gelu(x, approximate=True)
def _silu(x):
    return jax.nn.silu(x)
def _sigmoid(x):
    return jax.nn.sigmoid(x)
def _layernorm(x, axis=-1, eps=1e-5):
    m = jnp.mean(x, axis=axis, keepdims=True)
    v = jnp.var(x, axis=axis, keepdims=True)
    return (x - m) / jnp.sqrt(v + eps)
def _scatter_add(tgt, idx, src, axis=0):
    return tgt.at[idx].add(src)
def _segment_sum(src, seg, n):
    return jax.ops.segment_sum(src, seg, n)
class _Rng:
    def __init__(self, key):
        self._k = key
    def _next(self):
        self._k, sub = jax.random.split(self._k)
        return sub
    def normal(self, shape):
        return jax.random.normal(self._next(), shape, dtype=jnp.bfloat16)
    def randint(self, lo, hi, shape):
        return jax.random.randint(self._next(), shape, lo, hi, dtype=jnp.int32)
    def uniform(self, shape, lo=0.0, hi=1.0):
        return jax.random.uniform(self._next(), shape, jnp.bfloat16, lo, hi)
    def permutation(self, n):
        return jax.random.permutation(self._next(), n)


kernel_name = 'gated_mix__softmax_full_mha__dense_activation_squared_relu__prompt'

def setup_inputs():
    _rng = _Rng(jax.random.key(int.from_bytes(__import__("os").urandom(4), "little")))
    _w = (lambda a: (lambda t: t.astype(jnp.bfloat16) if jnp.issubdtype(t.dtype, jnp.floating) else t)(jnp.asarray(a)))
    def _A_setup():
        B, S, D = 1, 2048, 640
        return {
            "x": _w((lambda *s: _rng.normal(s) * 0.05)(B, S, D)),
            "wqkv": _w((lambda *s: _rng.normal(s) * 0.4)(D, 3 * D)),
            "wo": _w((lambda *s: _rng.normal(s) * 0.05)(D, D)),
        }
    _A_in = _A_setup()

    def _B_setup():
        B, S, D, F = 1, 2048, 640, 1536
        return {
            "x": _w((lambda *s: _rng.normal(s) * 0.05)(B, S, D)),
            "w1": _w((lambda *s: _rng.normal(s) * 0.05)(D, F)),
            "b1": _w((lambda *s: _rng.normal(s) * 0.05)(F)),
            "w2": _w((lambda *s: _rng.normal(s) * 0.05)(F, D)),
            "b2": _w((lambda *s: _rng.normal(s) * 0.05)(D)),
        }
    _B_in = _B_setup()

    return {
        "A_x": _A_in["x"],
        "A_wqkv": _A_in["wqkv"],
        "A_wo": _A_in["wo"],
        "B_x": _B_in["x"],
        "B_w1": _B_in["w1"],
        "B_b1": _B_in["b1"],
        "B_w2": _B_in["w2"],
        "B_b2": _B_in["b2"],
        "gate_w": _w((lambda *s: _rng.normal(s) * 0.05)(640) * 16.0),
    }

def reference(A_x, A_wqkv, A_wo, B_x, B_w1, B_b1, B_w2, B_b2, gate_w):
    def _A_ref(x, wqkv, wo):
        B, S, D = x.shape
        H = 32; Dh = D // H
        qkv = (lambda x, *d: x.transpose(*d))((x @ wqkv).reshape(B, S, 3, H, Dh), 2, 0, 3, 1, 4)
        q, k, v = qkv[0], qkv[1], qkv[2]
        scale = Dh ** -0.5
        scores = jnp.einsum("bhqd,bhkd->bhqk", q, k) * scale
        p = _softmax(scores, axis=-1)
        o = jnp.einsum("bhqk,bhkd->bhqd", p, v)
        return (lambda x, *d: x.transpose(*d))(o, 0, 2, 1, 3).reshape(B, S, D) @ wo

    def _B_ref(x, w1, b1, w2, b2):
        h = jnp.einsum("bsd,df->bsf", x, w1) + b1
        zero = jnp.zeros_like(h)
        r = jnp.where(h > zero, h, zero)
        h = r * r
        out = jnp.einsum("bsf,fd->bsd", h, w2) + b2
        return out

    x = A_x
    g = _sigmoid((x * gate_w).sum(-1, keepdims=True))
    a = _A_ref(x, A_wqkv, A_wo)
    b = _B_ref(x, B_w1, B_b1, B_w2, B_b2)
    return g * a + (1 - g) * b
```

```python
import functools
import math

import jax
import jax.numpy as jnp
from jax import lax
import jax.experimental.pallas as pl
import jax.experimental.pallas.tpu as pltpu

H = 32
LANES = 128
TQ = 512
KC = 128
LAG = 2
UPI = 8
RC = 512

NT = (((1,), (1,)), ((), ()))
NN = (((1,), (0,)), ((), ()))
TN = (((0,), (0,)), ((), ()))
F32 = jnp.float32
BF16 = jnp.bfloat16


def _kernel(x_ref, wqkv_ref, wo_ref, w1_ref, b1_ref, w2_ref, b2_ref, gw_ref,
            o_ref,
            q_ref, k_ref, vt_ref, ot_ref, s0, s1, m0, m1, *, S, D, DH):
    NG = D // LANES
    NQ = S // TQ
    U = H * NQ
    NKC = S // KC
    qscale = (DH ** -0.5) * math.log2(math.e)

    lane_rc = lax.broadcasted_iota(jnp.int32, (RC, LANES), 1)
    row24_rc = lax.broadcasted_iota(jnp.int32, (24, RC), 0)
    wvT = wqkv_ref[:, 2 * D:3 * D].astype(F32).T.astype(BF16)
    for r in range(S // RC):
        rows = slice(r * RC, (r + 1) * RC)
        xc = x_ref[rows, :]
        qk = jnp.dot(xc, wqkv_ref[:, 0:2 * D], preferred_element_type=F32)
        for (ref, base, sc) in ((q_ref, 0, qscale), (k_ref, D, None)):
            grp = []
            for g in range(NG):
                t = qk[:, base + g * LANES: base + (g + 1) * LANES]
                if sc is not None:
                    t = t * sc
                grp.append(t)
                ref[g, rows, :] = t.astype(BF16)
            for g in range(NG - 1):
                ref[NG + g, rows, :] = jnp.where(lane_rc >= LANES // 2, grp[g], grp[g + 1]).astype(BF16)
        vT = lax.dot_general(wvT, xc, NT, preferred_element_type=F32)
        vT = vT.astype(BF16).astype(F32)
        for h in range(H):
            odd = h % 2
            off = 2 * DH * (h // 2) + 16 * odd
            win = vT[off:off + 24, :]
            valid = (row24_rc >= 4) if odd else (row24_rc < DH)
            vt_ref[h, :, rows] = jnp.where(valid, win, 1.0)

    lane = lax.broadcasted_iota(jnp.int32, (TQ, LANES), 1)
    row8 = lax.broadcasted_iota(jnp.int32, (8, TQ), 0)
    sb = (s0, s1)
    mb = (m0, m1)

    def a_init(u):
        h = u // NQ
        qt = u % NQ
        lo = h * DH
        ga = lo // LANES
        gb = (lo + DH - 1) // LANES
        g = jnp.where(ga == gb, ga, NG + ga)
        q = q_ref[g, pl.ds(pl.multiple_of(qt * TQ, TQ), TQ), :]
        msk = ((lane - lo) & (LANES - 1)) < DH
        qm = jnp.where(msk, q.astype(F32), 0.0).astype(BF16)
        return g, qm

    def a_chunk(info, c, m, s_ref):
        g, qm = info
        kc = k_ref[g, c * KC:(c + 1) * KC, :]
        s = lax.dot_general(kc, qm, NT, preferred_element_type=F32)
        s_ref[c * KC:(c + 1) * KC, :] = s
        mc = jnp.max(s.reshape(KC // 8, 8, TQ), axis=0)
        return mc if m is None else jnp.maximum(m, mc)

    def a_fin(m, m_ref):
        m = jnp.max(m, axis=0, keepdims=True)
        m_ref[...] = jnp.broadcast_to(m, (8, TQ))

    def b_chunk(h, m, c, acc, s_ref):
        p = jnp.exp2(s_ref[c * KC:(c + 1) * KC, :] - m).astype(BF16)
        vt = vt_ref[h, :, c * KC:(c + 1) * KC]
        a = lax.dot_general(vt, p, NN, preferred_element_type=F32)
        return a if acc is None else acc + a

    info = a_init(0)
    m = None
    for c in range(NKC):
        m = a_chunk(info, c, m, s0)
    a_fin(m, m0)
    info = a_init(1)
    m = None
    for c in range(LAG):
        m = a_chunk(info, c, m, s1)

    assert UPI == 2 * NQ

    def body(i, m):
        u0 = UPI * i
        info = None
        even_o = {}
        for j in range(UPI):
            odd = j // NQ
            qt = j % NQ
            hb = 2 * i + odd
            mb_v = mb[j % 2][0:1, :]
            acc = None
            for c in range(NKC):
                ta = c + LAG
                ja = j + 1 + ta // NKC
                ca = ta % NKC
                if info is None or ca == 0:
                    info = a_init(jnp.minimum(u0 + ja, U - 1))
                    if ca == 0:
                        m = None
                m = a_chunk(info, ca, m, sb[ja % 2])
                if ca == NKC - 1:
                    a_fin(m, mb[ja % 2])
                acc = b_chunk(hb, mb_v, c, acc, sb[j % 2])
            l = acc[0:1] if odd else acc[23:24]
            o = acc * (1.0 / l)
            base = pl.multiple_of(2 * DH * i, 8)
            cols = slice(qt * TQ, (qt + 1) * TQ)
            if not odd:
                ot_ref[pl.ds(base, 24), cols] = o
            else:
                off = pl.multiple_of(base + 16, 8)
                old = ot_ref[pl.ds(off, 8), cols]
                ot_ref[pl.ds(off, 8), cols] = jnp.where(row8 >= 4, o[0:8], old)
                ot_ref[pl.ds(off + 8, 16), cols] = o[8:24]
        return m

    lax.fori_loop(0, U // UPI, body, m)

    b1 = b1_ref[...].astype(F32)
    b2 = b2_ref[...].astype(F32)
    gw = gw_ref[...].astype(F32)
    for r in range(S // RC):
        rows = slice(r * RC, (r + 1) * RC)
        xc = x_ref[rows, :]
        o = ot_ref[:, rows].T.astype(BF16)
        a = jnp.dot(o, wo_ref[...], preferred_element_type=F32)
        hh = jnp.dot(xc, w1_ref[...], preferred_element_type=F32) + b1
        hh = jnp.maximum(hh, 0.0)
        hh = (hh * hh).astype(BF16)
        b = jnp.dot(hh, w2_ref[...], preferred_element_type=F32) + b2
        z = jnp.sum(xc.astype(F32) * gw, axis=-1, keepdims=True)
        g = 1.0 / (1.0 + jnp.exp(-z))
        o_ref[rows, :] = (g * a + (1.0 - g) * b).astype(o_ref.dtype)


@jax.jit
def pallas_gated_mix__softmax_full_mha__dense_activation_squared_relu__prompt_kernel(
    A_x, A_wqkv, A_wo, B_x, B_w1, B_b1, B_w2, B_b2, gate_w,
):
    B, S, D = A_x.shape
    assert B == 1
    F = B_w1.shape[1]
    DH = D // H
    NG = D // LANES
    x = A_x.reshape(S, D)
    out = pl.pallas_call(
        functools.partial(_kernel, S=S, D=D, DH=DH),
        out_shape=jax.ShapeDtypeStruct((S, D), A_x.dtype),
        scratch_shapes=[
            pltpu.VMEM((2 * NG - 1, S, LANES), BF16),
            pltpu.VMEM((2 * NG - 1, S, LANES), BF16),
            pltpu.VMEM((H, 24, S), F32),
            pltpu.VMEM((D, S), F32),
            pltpu.VMEM((S, TQ), F32),
            pltpu.VMEM((S, TQ), F32),
            pltpu.VMEM((8, TQ), F32),
            pltpu.VMEM((8, TQ), F32),
        ],
        compiler_params=pltpu.CompilerParams(vmem_limit_bytes=100 * 1024 * 1024),
    )(x, A_wqkv, A_wo, B_w1, B_b1.reshape(1, F), B_w2, B_b2.reshape(1, D), gate_w.reshape(1, D))
    return out.reshape(B, S, D)
```

```python
import functools
import math

import jax
import jax.numpy as jnp
from jax import lax
import jax.experimental.pallas as pl
import jax.experimental.pallas.tpu as pltpu

H = 32
LANES = 128
TQ = 512
KC = 128
VR = 16
LAG = 2
NCH = 2
RC = 512
SAFE_LOG2 = 40.0
FORCE = 0
NIT = 16
QVN = 128
UN3 = 0
FEARLY = 1

NT = (((1,), (1,)), ((), ()))
NN = (((1,), (0,)), ((), ()))
F32 = jnp.float32
BF16 = jnp.bfloat16
U32 = jnp.uint32


def _qw_tiles(h, DH):
    lo = h * DH
    out = []
    for t0 in range(0, LANES, 16):
        src = [lo + ((t0 + e - lo) % LANES) for e in range(16)]
        ok = [r < lo + DH for r in src]
        if not any(ok):
            out.append(None)
        else:
            e0 = ok.index(True)
            out.append((src[e0] - e0, e0, e0 + sum(ok)))
    return out


def _kernel(x_hbm, wqkv_hbm, wo_hbm, w1_hbm, b1_ref, w2_hbm, b2_ref, gw_ref,
            o_hbm,
            x_ref, wqkv_ref, wo_ref, w1_ref, w2_ref, o_ref,
            qt_ref, k_ref, vt_ref, ot_ref, fb_ref, kb_ref, qb_ref, qw_ref,
            mk_ref, in_sem, x_sem, out_sem, *, S, D, DH):
    NG = D // LANES
    NQ = S // TQ
    NKC = S // KC
    NR = S // RC
    NP = H // 2
    FC = S // NP
    NJ = TQ // LANES
    qscale = (DH ** -0.5) * math.log2(math.e)

    def chunk(r, n=RC):
        return pl.ds(pl.multiple_of(r * n, n), n)

    def wcopy(n):
        return pltpu.make_async_copy(wqkv_hbm.at[:, pl.ds(n * D, D)], wqkv_ref.at[n], in_sem.at[n])

    def xcopy(r):
        return pltpu.make_async_copy(x_hbm.at[0, chunk(r), :], x_ref.at[chunk(r), :], x_sem.at[r])

    cp_wq, cp_wk, cp_wv = wcopy(0), wcopy(1), wcopy(2)
    cp_w1 = pltpu.make_async_copy(w1_hbm, w1_ref, in_sem.at[3])
    cp_w2 = pltpu.make_async_copy(w2_hbm, w2_ref, in_sem.at[4])
    cp_wo = pltpu.make_async_copy(wo_hbm, wo_ref, in_sem.at[5])
    for cp in [xcopy(0), cp_wk] + [xcopy(r) for r in range(1, NR)] + [cp_wq, cp_wv, cp_w1, cp_w2, cp_wo]:
        cp.start()

    for h in range(H):
        for t, info in enumerate(_qw_tiles(h, DH)):
            if info is None:
                qw_ref[h, 8 * t:8 * t + 8, :] = jnp.zeros((8, S), U32)
    mk_ref[...] = jnp.zeros(mk_ref.shape, F32)

    def group(h):
        lo = h * DH
        ga = lo // LANES
        gb = (lo + DH - 1) // LANES
        return lo, jnp.where(ga == gb, ga, NG + ga)

    def prep(pair, never):
        base = pl.multiple_of(2 * DH * pair, 8)
        links = []
        for odd in range(2):
            lo, g = group(2 * pair + odd)
            src = jnp.concatenate(
                [k_ref[g, c * (KC // 2):c * (KC // 2) + VR // 2, :] for c in range(NKC)], axis=0)
            for d in range(DH):
                idx = jnp.zeros(src.shape, jnp.int32) + ((lo + d) & (LANES - 1))
                kb = jnp.take_along_axis(src, idx, axis=1, mode="promise_in_bounds")
                kb = pltpu.bitcast(kb, BF16).astype(F32)
                kb_ref[odd, d] = kb
                links += [kb[0:8], kb[128:136]]
        if never is None:
            return
        n = 0
        for t in range(2 * DH // 8):
            for j in range(S // LANES):
                win = qt_ref[pl.ds(base + 8 * t, 8), j * LANES:(j + 1) * LANES]
                win = jnp.where(never, links[n], win)
                n += 1
                for r in range(8):
                    qb_ref[8 * t + r, :, j * LANES:(j + 1) * LANES] = jnp.broadcast_to(win[r:r + 1, :], (8, LANES))

    def prep_q(pair):
        win = qt_ref[pl.ds(pl.multiple_of(2 * DH * pair, 8), 2 * DH), :]
        for r in range(2 * DH):
            qb_ref[r] = jnp.broadcast_to(win[r:r + 1, :], (8, S))

    lane_rc = lax.broadcasted_iota(jnp.int32, (RC, LANES), 1)
    row24_rc = lax.broadcasted_iota(jnp.int32, (24, RC), 0)
    row16_rc = lax.broadcasted_iota(jnp.int32, (16, RC), 0)

    def lane_fold_absmax(a):
        a = jnp.abs(a)
        out = a[:, 0:LANES]
        for j in range(1, a.shape[1] // LANES):
            out = jnp.maximum(out, a[:, j * LANES:(j + 1) * LANES])
        return out

    cp_wk.wait()

    def proj_k(r, c):
        xcopy(r).wait()
        k = jnp.dot(x_ref[chunk(r), :], wqkv_ref[1], preferred_element_type=F32)
        grp = [k[:, g * LANES:(g + 1) * LANES] for g in range(NG)]
        grp += [jnp.where(lane_rc >= LANES // 2, grp[g], grp[g + 1]) for g in range(NG - 1)]
        for g, t in enumerate(grp):
            k_ref[g, chunk(r, RC // 2), :] = pltpu.bitcast(t.astype(BF16), U32)
        mk_ref[...] = jnp.maximum(mk_ref[...], jnp.max(jnp.abs(k).reshape(RC // 8, 8, D), axis=0))
        return c

    lax.fori_loop(0, NR, proj_k, 0)
    cp_wq.wait()
    cp_wv.wait()

    mk = jnp.max(mk_ref[...], axis=0, keepdims=True)
    col = lax.broadcasted_iota(jnp.int32, (H, D), 1)
    hrow = lax.broadcasted_iota(jnp.int32, (H, D), 0) * DH
    sel = jnp.where((col >= hrow) & (col < hrow + DH), mk, 0.0)

    def proj_qv(r, carry):
        bnd, mv = carry
        rows = chunk(r)
        xc = x_ref[rows, :]
        qs, vs = [], []
        for j0 in range(0, D, QVN):
            j1 = min(j0 + QVN, D)
            q = jnp.dot(xc, wqkv_ref[0, :, j0:j1], preferred_element_type=F32)
            qs.append((q * qscale).astype(BF16).astype(F32).T)
            v = jnp.dot(xc, wqkv_ref[2, :, j0:j1], preferred_element_type=F32)
            vs.append(v.astype(BF16).astype(F32).T)
        qT = jnp.concatenate(qs, axis=0)
        vT = jnp.concatenate(vs, axis=0)
        qt_ref[:, rows] = qT
        for h in range(H):
            for t, info in enumerate(_qw_tiles(h, DH)):
                if info is not None:
                    base, e0, e1 = info
                    w = qT[base:base + 16, :]
                    if e1 - e0 < 16:
                        w = jnp.where((row16_rc >= e0) & (row16_rc < e1), w, 0.0)
                    qw_ref[h, 8 * t:8 * t + 8, rows] = pltpu.bitcast(w.astype(BF16), U32)
            odd = h % 2
            off = 2 * DH * (h // 2) + 16 * odd
            valid = (row24_rc >= 4) if odd else (row24_rc < DH)
            vt_ref[h, :, rows] = jnp.where(valid, vT[off:off + 24, :], 1.0)
        b = jnp.dot(sel, lane_fold_absmax(qT), preferred_element_type=F32)
        bnd = jnp.maximum(bnd, jnp.max(b.reshape(H // 8, 8, LANES), axis=0))
        mv = jnp.maximum(mv, jnp.max(lane_fold_absmax(vT).reshape(D // 8, 8, LANES), axis=0))
        return bnd, mv

    zero8 = jnp.zeros((8, LANES), F32)
    carry = proj_qv(0, (zero8, zero8))
    prep(0, None)
    bnd, mv = lax.fori_loop(1, NR, proj_qv, carry)
    bound = jnp.max(bnd)
    vmax = jnp.max(mv)
    safe = (bound <= SAFE_LOG2) & (vmax <= 2.0 ** 60) & (vmax >= 2.0 ** -60)
    if FORCE == 1:
        safe = bound > -1.0
    if FORCE == 2:
        safe = bound < -1.0

    cp_w1.wait()
    cp_w2.wait()
    b1 = b1_ref[...].astype(F32).reshape(1, -1)
    b2 = b2_ref[...].astype(F32).reshape(1, -1)

    def ffn1(rows):
        hh = jnp.dot(x_ref[rows, :], w1_ref[...], preferred_element_type=F32) + b1
        hh = jnp.maximum(hh, 0.0)
        return (hh * hh).astype(BF16)

    def ffn2(rows, hh):
        fb_ref[rows, :] = jnp.dot(hh, w2_ref[...], preferred_element_type=F32) + b2

    row8 = lax.broadcasted_iota(jnp.int32, (8, TQ), 0)

    def store_o(acc, pair, odd, cols):
        l = acc[0:1] if odd else acc[23:24]
        o = acc * (1.0 / l)
        base = pl.multiple_of(2 * DH * pair, 8)
        if not odd:
            ot_ref[pl.ds(base, 24), cols] = o
        else:
            off = pl.multiple_of(base + 16, 8)
            old = ot_ref[pl.ds(off, 8), cols]
            ot_ref[pl.ds(off, 8), cols] = jnp.where(row8 >= 4, o[0:8], old)
            ot_ref[pl.ds(off + 8, 16), cols] = o[8:24]

    @pl.when(safe)
    def _fast():
        never = bnd < 0.0
        prep_q(0)

        def p_tile(h, g, odd, qt, c):
            kc = pltpu.bitcast(k_ref[g, c * (KC // 2) + VR // 2:(c + 1) * (KC // 2), :], BF16)
            accs = [[None] * NJ for _ in range(VR // 8)]
            items = [(r, j) for j in range(NJ) for r in range(VR // 8)]
            prev = None
            for k0 in range(0, len(items), NCH):
                grp = items[k0:k0 + NCH]
                for d in range(DH):
                    for n, (r, j) in enumerate(grp):
                        kbv = kb_ref[odd, d, c * VR + 8 * r:c * VR + 8 * r + 8, :]
                        qbv = qb_ref[odd * DH + d, :, qt * TQ + j * LANES:qt * TQ + (j + 1) * LANES]
                        t = kbv * qbv
                        if d == 0 and prev is not None:
                            t = jnp.where(never, prev[n], t)
                        accs[r][j] = t if accs[r][j] is None else accs[r][j] + t
                prev = [accs[r][j] for (r, j) in grp]
            sv = jnp.concatenate([jnp.concatenate(a, axis=1) for a in accs], axis=0)
            w = pltpu.bitcast(qw_ref[h, :, qt * TQ:(qt + 1) * TQ], BF16)
            sm = lax.dot_general(kc, w, NN, preferred_element_type=F32)
            return jnp.exp2(jnp.concatenate([sv, sm], axis=0))

        def body(i, carry):
            T = 2 * NQ * NKC
            gs = [group(2 * i + odd)[1] for odd in range(2)]
            rows = chunk(i, FC)
            ps = {}
            acc = None
            hh = None
            for t in range(T + LAG):
                if t < T:
                    u, c = divmod(t, NKC)
                    odd, qt = divmod(u, NQ)
                    ps[t] = p_tile(2 * i + odd, gs[odd], odd, qt, c)
                if t == T and FEARLY:
                    hh = ffn1(rows)
                tb = t - LAG
                if tb >= 0:
                    u, c = divmod(tb, NKC)
                    odd, qt = divmod(u, NQ)
                    vt = vt_ref[2 * i + odd, :, c * KC:(c + 1) * KC]
                    a = lax.dot_general(vt, ps.pop(tb).astype(BF16), NN, preferred_element_type=F32)
                    acc = a if c == 0 else acc + a
                    if c == NKC - 1:
                        store_o(acc, i, odd, slice(qt * TQ, (qt + 1) * TQ))
            if hh is None:
                hh = ffn1(rows)
            ffn2(rows, hh)
            prep(jnp.minimum(i + 1, NP - 1), never)
            return carry

        lax.fori_loop(0, NIT, body, 0)

    @pl.when(jnp.logical_not(safe))
    def _slow():
        def body(i, carry):
            for odd in range(2):
                h = 2 * i + odd
                g = group(h)[1]

                def unit(qt, c2):
                    cols = chunk(qt, TQ)
                    w = pltpu.bitcast(qw_ref[h, :, cols], BF16)
                    s = lax.dot_general(pltpu.bitcast(k_ref[g], BF16), w, NN, preferred_element_type=F32)
                    m = jnp.max(s, axis=0, keepdims=True)
                    p = jnp.exp2(s - m).astype(BF16)
                    acc = lax.dot_general(vt_ref[h], p, NN, preferred_element_type=F32)
                    store_o(acc, i, odd, cols)
                    return c2

                lax.fori_loop(0, NQ, unit, 0)
            rows = chunk(i, FC)
            ffn2(rows, ffn1(rows))
            return carry

        lax.fori_loop(0, NP, body, 0)

    cp_wo.wait()
    gw = gw_ref[...].astype(F32).reshape(1, -1)

    def out_copy(r):
        return pltpu.make_async_copy(o_ref.at[chunk(r), :], o_hbm.at[0, chunk(r), :], out_sem.at[r])

    def p3(r, c):
        rows = chunk(r)
        o = ot_ref[:, rows].T.astype(BF16)
        a = jnp.dot(o, wo_ref[...], preferred_element_type=F32)
        z = jnp.sum(x_ref[rows, :].astype(F32) * gw, axis=-1, keepdims=True)
        g = 1.0 / (1.0 + jnp.exp(-z))
        o_ref[rows, :] = (g * a + (1.0 - g) * fb_ref[rows, :]).astype(o_ref.dtype)
        out_copy(r).start()
        return c

    if UN3:
        for r in range(NR):
            p3(r, 0)
    else:
        lax.fori_loop(0, NR, p3, 0)
    for r in range(NR):
        out_copy(r).wait()


@jax.jit
def pallas_gated_mix__softmax_full_mha__dense_activation_squared_relu__prompt_kernel(
    A_x, A_wqkv, A_wo, B_x, B_w1, B_b1, B_w2, B_b2, gate_w,
):
    B, S, D = A_x.shape
    assert B == 1
    F = B_w1.shape[1]
    DH = D // H
    NG = D // LANES
    hbm = pl.BlockSpec(memory_space=pl.ANY)
    vmem = pl.BlockSpec(memory_space=pltpu.VMEM)
    return pl.pallas_call(
        functools.partial(_kernel, S=S, D=D, DH=DH),
        out_shape=jax.ShapeDtypeStruct((B, S, D), A_x.dtype),
        in_specs=[hbm, hbm, hbm, hbm, vmem, hbm, vmem, vmem],
        out_specs=hbm,
        scratch_shapes=[
            pltpu.VMEM((S, D), BF16),
            pltpu.VMEM((3, D, D), BF16),
            pltpu.VMEM((D, D), BF16),
            pltpu.VMEM((D, F), BF16),
            pltpu.VMEM((F, D), BF16),
            pltpu.VMEM((S, D), BF16),
            pltpu.VMEM((D, S), F32),
            pltpu.VMEM((2 * NG - 1, S // 2, LANES), U32),
            pltpu.VMEM((H, 24, S), F32),
            pltpu.VMEM((D, S), F32),
            pltpu.VMEM((S, D), F32),
            pltpu.VMEM((2, DH, (S // KC) * VR, LANES), F32),
            pltpu.VMEM((2 * DH, 8, S), F32),
            pltpu.VMEM((H, LANES // 2, S), U32),
            pltpu.VMEM((8, D), F32),
            pltpu.SemaphoreType.DMA((6,)),
            pltpu.SemaphoreType.DMA((S // RC,)),
            pltpu.SemaphoreType.DMA((S // RC,)),
        ],
        compiler_params=pltpu.CompilerParams(vmem_limit_bytes=120 * 1024 * 1024),
    )(A_x, A_wqkv, A_wo, B_w1, B_b1, B_w2, B_b2, gate_w)
```

```python
import functools
import math

import jax
import jax.numpy as jnp
from jax import lax
import jax.experimental.pallas as pl
import jax.experimental.pallas.tpu as pltpu

H = 32
LANES = 128
TQ = 512
KC = 128
VR = 16
XT = 2
LAG = 2
SA = 2
DC = 4
RC = 512
TS = 256
F1A = 512
NLH = 32
OUT_CHUNKS = (512, 512, 512, 256, 128, 128)
SAFE_LOG2 = 40.0

NN = (((1,), (0,)), ((), ()))
F32 = jnp.float32
BF16 = jnp.bfloat16
U32 = jnp.uint32


def _kernel(x_hbm, wqkv_hbm, wo_hbm, w1_hbm, b1_hbm, w2_hbm, b2_hbm, gw_hbm,
            o_hbm,
            x_ref, wqkv_ref, wo_ref, w1_ref, w2_ref, o_ref,
            qt_ref, k_ref, vt_ref, ot_ref, fb_ref, kb_ref, qb_ref, qw_ref,
            mk_ref, mq_ref, b1_ref, b2_ref, gw_ref, in_sem, x_sem, out_sem, *, S, D, DH):
    NG = D // LANES
    NQ = S // TQ
    NKC = S // KC
    NR = S // RC
    NP = H // 2
    PW = 2 * DH
    FC = S // NP
    NJ = TQ // LANES
    FF = w1_ref.shape[1]
    KH = KC // 2
    qscale = (DH ** -0.5) * math.log2(math.e)
    xtiles = [(e + 1) * NKC // XT - 1 for e in range(XT)]
    assert 2 * NJ * XT == NKC

    def chunk(r, n=RC):
        return pl.ds(pl.multiple_of(r * n, n), n)

    def wcopy(n):
        return pltpu.make_async_copy(wqkv_hbm.at[:, pl.ds(n * D, D)], wqkv_ref.at[n], in_sem.at[n])

    def xcopy(r):
        return pltpu.make_async_copy(x_hbm.at[0, chunk(r), :], x_ref.at[chunk(r), :], x_sem.at[r])

    cp_wq, cp_wk, cp_wv = wcopy(0), wcopy(1), wcopy(2)
    cp_late = [pltpu.make_async_copy(a, b, in_sem.at[3 + n]) for n, (a, b) in enumerate((
        (w1_hbm, w1_ref), (w2_hbm, w2_ref), (wo_hbm, wo_ref),
        (b1_hbm, b1_ref), (b2_hbm, b2_ref), (gw_hbm, gw_ref)))]
    xcopy(0).start()
    cp_wk.start()
    mk_ref[...] = jnp.zeros(mk_ref.shape, F32)
    mq_ref[...] = jnp.zeros(mq_ref.shape, F32)

    def prep(pair, never, pace, n_pace):
        src = jnp.concatenate(
            [k_ref[pair, c * KH:c * KH + VR // 2, :] for c in range(NKC)]
            + [k_ref[pair, c * KH + VR // 2:c * KH + VR, :] for c in xtiles], axis=0)
        kpace = []
        for d in range(PW):
            kb = jnp.broadcast_to(src[:, d:d + 1], src.shape)
            kb_ref[d] = pltpu.bitcast(kb, BF16).astype(F32)
            kpace.append(kb[0:8])
        base = pl.multiple_of(PW * pair, 8)
        nt = (PW // 8) * (S // LANES)
        n = 0
        for t in range(PW // 8):
            for j in range(S // LANES):
                win = qt_ref[pl.ds(base + 8 * t, 8), j * LANES:(j + 1) * LANES]
                if n < n_pace:
                    after = pace[n * len(pace) // n_pace]
                else:
                    after = kpace[(n - n_pace) * PW // (nt - n_pace)]
                win = jnp.where(never, pltpu.bitcast(after, F32), win)
                n += 1
                qb_ref[8 * t:8 * t + 8, :, j * LANES:(j + 1) * LANES] = jnp.stack(
                    [jnp.broadcast_to(win[r:r + 1, :], (8, LANES)) for r in range(8)])

    def lane_fold_absmax(a):
        a = jnp.abs(a)
        out = a[:, 0:LANES]
        for j in range(1, a.shape[1] // LANES):
            out = jnp.maximum(out, a[:, j * LANES:(j + 1) * LANES])
        return out

    cp_wk.wait()
    for cp in [xcopy(r) for r in range(1, NR)] + [cp_wq, cp_wv]:
        cp.start()

    def proj_k(r, c):
        xcopy(r).wait()
        lane = lax.broadcasted_iota(jnp.int32, (RC // 2, LANES), 1)
        mk = mk_ref[...]
        k = jnp.dot(x_ref[chunk(r), :], wqkv_ref[1], preferred_element_type=F32)
        kp = pltpu.bitcast(k.astype(BF16), U32)
        grp = [kp[:, g * LANES:(g + 1) * LANES] for g in range(NG)]
        for p in range(NP):
            g, off = divmod(PW * p, LANES)
            t = grp[g]
            if off + PW > LANES:
                t = jnp.where(lane >= off, t, grp[g + 1])
            if off:
                t = pltpu.roll(t, LANES - off, 1)
            k_ref[p, chunk(r, RC // 2), :] = t
        mk_ref[...] = jnp.maximum(mk, jnp.max(jnp.abs(k).reshape(RC // 8, 8, D), axis=0))
        return c

    lax.fori_loop(0, NR, proj_k, 0)
    for cp in cp_late:
        cp.start()
    cp_wq.wait()
    cp_wv.wait()

    row24 = lax.broadcasted_iota(jnp.int32, (24, RC), 0)

    def proj_qv(r, mv, pace=None):
        rows = chunk(r)
        xc = x_ref[rows, :]
        qs, vs = [], []
        for j0 in range(0, D, LANES):
            q = jnp.dot(xc, wqkv_ref[0, :, j0:j0 + LANES], preferred_element_type=F32)
            qs.append((q * qscale).astype(BF16).astype(F32).T)
        for j0 in range(0, D, LANES):
            v = jnp.dot(xc, wqkv_ref[2, :, j0:j0 + LANES], preferred_element_type=F32)
            vs.append(v.astype(BF16).astype(F32).T)
            if pace is not None and j0 < D - LANES:
                pace += [v[r_:r_ + 8] for r_ in range(0, RC, 8)]
        qT = jnp.concatenate(qs, axis=0)
        vT = jnp.concatenate(vs, axis=0)
        qt_ref[:, rows] = qT
        zero8 = jnp.zeros((8, RC), F32)
        for h in range(H):
            odd = h % 2
            off = PW * (h // 2) + 16 * odd
            valid = (row24 >= 4) if odd else (row24 < DH)
            w = jnp.concatenate([jnp.where(valid, qT[off:off + 24, :], 0.0), zero8], axis=0)
            qw_ref[h, :, rows] = pltpu.bitcast(w.astype(BF16), U32)
            vt_ref[h, :, rows] = jnp.where(valid, vT[off:off + 24, :], 1.0)
        mq_ref[...] = jnp.maximum(mq_ref[...], lane_fold_absmax(qT))
        return jnp.maximum(mv, jnp.max(lane_fold_absmax(vT).reshape(D // 8, 8, LANES), axis=0))

    mv = lax.fori_loop(0, NR - 1, proj_qv, jnp.zeros((8, LANES), F32))
    for cp in cp_late:
        cp.wait()
    never0 = mv < 0.0
    pace0 = []
    mv = proj_qv(NR - 1, mv, pace0)
    prep(0, never0, pace0, (PW // 8) * (S // LANES))

    mk = jnp.max(mk_ref[...], axis=0, keepdims=True)
    col = lax.broadcasted_iota(jnp.int32, (H, D), 1)
    hrow = lax.broadcasted_iota(jnp.int32, (H, D), 0) * DH
    sel = jnp.where((col >= hrow) & (col < hrow + DH), mk, 0.0)
    bnd = jnp.dot(sel, mq_ref[...], preferred_element_type=F32)
    bnd = jnp.max(bnd.reshape(H // 8, 8, LANES), axis=0)
    vmax = jnp.max(mv)
    safe = (jnp.max(bnd) <= SAFE_LOG2) & (vmax <= 2.0 ** 60) & (vmax >= 2.0 ** -60)

    def ffn1(rows, c0, c1):
        b1 = b1_ref[...].astype(F32).reshape(1, -1)
        hh = jnp.dot(x_ref[rows, :], w1_ref[:, c0:c1], preferred_element_type=F32) + b1[:, c0:c1]
        hh = jnp.maximum(hh, 0.0)
        return pltpu.bitcast((hh * hh).astype(BF16), U32)

    def ffn2(rows, hh):
        b2 = b2_ref[...].astype(F32).reshape(1, -1)
        fb_ref[rows, :] = jnp.dot(pltpu.bitcast(hh, BF16), w2_ref[...], preferred_element_type=F32) + b2

    def scores_mxu(kc, h, odd, cols, width):
        w = qw_ref[h, :, cols]
        if odd:
            w = jnp.concatenate([jnp.zeros((8, width), U32), w], axis=0)
        w = pltpu.bitcast(w, BF16)
        return lax.dot_general(pltpu.bitcast(kc, BF16)[:, 0:w.shape[0]], w, NN, preferred_element_type=F32)

    def store_o(acc, pair, odd, cols):
        l = acc[0:1] if odd else acc[23:24]
        o = acc * (1.0 / l)
        base = pl.multiple_of(PW * pair, 8)
        if not odd:
            ot_ref[pl.ds(base, 24), cols] = o
        else:
            row8 = lax.broadcasted_iota(jnp.int32, (8, acc.shape[1]), 0)
            off = pl.multiple_of(base + 16, 8)
            old = ot_ref[pl.ds(off, 8), cols]
            ot_ref[pl.ds(off, 8), cols] = jnp.where(row8 >= 4, o[0:8], old)
            ot_ref[pl.ds(off + 8, 16), cols] = o[8:24]

    @pl.when(safe)
    def _fast():
        never = bnd < 0.0
        bnd_acc = jnp.tile(bnd, (3, NJ))
        never_acc = bnd_acc < 0.0

        def after(x, dep):
            n = dep.shape[0]
            x0 = jnp.where(never[None], dep, x[0:n])
            return x0 if n == x.shape[0] else jnp.concatenate([x0, x[n:]], axis=0)

        def scores_vpu(odd, qt, r0, nr, j, start=None, mid=None):
            acc = None
            for m, d in enumerate(range(odd * DH, (odd + 1) * DH, DC)):
                kb = kb_ref[d:d + DC, r0:r0 + nr, :].reshape(DC, nr // 8, 8, LANES)
                qb = qb_ref[d:d + DC, :, qt * TQ + j * LANES:qt * TQ + (j + 1) * LANES]
                t = kb * qb[:, None]
                if acc is not None:
                    if m == 2 and mid is not None:
                        acc = after(acc, mid)
                    t = jnp.concatenate([acc[None], t], axis=0)
                elif start is not None:
                    t = jnp.concatenate([after(t[0], start)[None], t[1:]], axis=0)
                acc = jnp.sum(t, axis=0)
            return acc

        def p_vpu(odd, qt, c, extra):
            e, pos = divmod(c, 2 * NJ)
            side = scores_vpu(odd, qt, (NKC + e) * VR + 8 * (pos % 2), 8, pos // 2)
            extra.append(jnp.exp2(side[0]))
            cols = []
            for j in range(NJ):
                cols.append(scores_vpu(odd, qt, c * VR, VR, j, cols[-1] if cols else None,
                                       side if j == NJ - 1 else None))
            parts = [jnp.exp2(jnp.concatenate([a.reshape(VR, LANES) for a in cols], axis=1))]
            if c in xtiles:
                parts.append(jnp.concatenate(
                    [jnp.concatenate(extra[0::2], axis=1), jnp.concatenate(extra[1::2], axis=1)], axis=0))
                extra.clear()
            return parts

        def p_mxu(i, odd, qt, c, blocks):
            kc = jnp.concatenate([k_ref[i, c * KH + 8 * b:c * KH + 8 * b + 8, :] for b in blocks], axis=0)
            sm = jnp.exp2(scores_mxu(kc, 2 * i + odd, odd, slice(qt * TQ, (qt + 1) * TQ), TQ))
            return {b: sm[16 * n:16 * n + 16] for n, b in enumerate(blocks)}

        def body(i, carry):
            T = 2 * NQ * NKC
            rows = chunk(i, FC)
            ps = {}
            extra = []
            acc = bnd_acc
            for t in range(T + LAG):
                if t < T:
                    u, c = divmod(t, NKC)
                    odd, qt = divmod(u, NQ)
                    parts = p_vpu(odd, qt, c, extra)
                    blocks = list(range(KC // 16 - 1, len(parts) - 1, -1))
                    res = p_mxu(i, odd, qt, c, blocks[:SA])
                if t == T:
                    hh = ffn1(rows, 0, F1A)
                if t >= LAG:
                    ub, cb = divmod(t - LAG, NKC)
                    oddb, qtb = divmod(ub, NQ)
                    vt = vt_ref[2 * i + oddb, :, cb * KC:(cb + 1) * KC]
                    a = lax.dot_general(vt, ps.pop(t - LAG).astype(BF16), NN, preferred_element_type=F32)
                    acc = jnp.where(never_acc, acc, a) if cb == 0 else acc + a
                    if cb == NKC - 1:
                        store_o(acc, i, oddb, slice(qtb * TQ, (qtb + 1) * TQ))
                if t < T:
                    res.update(p_mxu(i, odd, qt, c, blocks[SA:]))
                    ps[t] = jnp.concatenate(parts + [res[b] for b in sorted(res)], axis=0)
            hh = jnp.concatenate([hh, ffn1(rows, F1A, FF)], axis=1)
            ffn2(rows, hh)
            pace = [hh[r:r + 8, c:c + LANES] for c in range(F1A, FF, LANES) for r in range(0, FC // 2, 8)]
            prep(jnp.minimum(i + 1, NP - 1), never, pace, NLH)
            return carry

        lax.fori_loop(0, NP, body, 0)

    @pl.when(jnp.logical_not(safe))
    def _fallback():
        def unit(u, carry):
            i = u // (S // TS)
            cols = chunk(u % (S // TS), TS)
            for odd in range(2):
                s = scores_mxu(k_ref[i], 2 * i + odd, odd, cols, TS)
                m = jnp.max(s, axis=0, keepdims=True)
                p = jnp.exp2(s - m).astype(BF16)
                acc = lax.dot_general(vt_ref[2 * i + odd], p, NN, preferred_element_type=F32)
                store_o(acc, i, odd, cols)
            return carry

        lax.fori_loop(0, NP * (S // TS), unit, 0)

        def ffn(i, carry):
            rows = chunk(i, 64)
            ffn2(rows, ffn1(rows, 0, FF))
            return carry

        lax.fori_loop(0, S // 64, ffn, 0)

    gw = gw_ref[...].astype(F32).reshape(1, -1)
    copies = []
    r0 = 0
    for n, sz in enumerate(OUT_CHUNKS):
        rows = pl.ds(r0, sz)
        r0 += sz
        o = ot_ref[:, rows].T.astype(BF16)
        a = jnp.dot(o, wo_ref[...], preferred_element_type=F32)
        z = jnp.sum(x_ref[rows, :].astype(F32) * gw, axis=-1, keepdims=True)
        g = 1.0 / (1.0 + jnp.exp(-z))
        o_ref[rows, :] = (g * a + (1.0 - g) * fb_ref[rows, :]).astype(o_ref.dtype)
        cp = pltpu.make_async_copy(o_ref.at[rows, :], o_hbm.at[0, rows, :], out_sem.at[n])
        cp.start()
        copies.append(cp)
    for cp in copies:
        cp.wait()


@jax.jit
def pallas_gated_mix__softmax_full_mha__dense_activation_squared_relu__prompt_kernel(
    A_x: jax.Array,
    A_wqkv: jax.Array,
    A_wo: jax.Array,
    B_x: jax.Array,
    B_w1: jax.Array,
    B_b1: jax.Array,
    B_w2: jax.Array,
    B_b2: jax.Array,
    gate_w: jax.Array,
):
    del B_x
    B, S, D = A_x.shape
    F = B_w1.shape[1]
    DH = D // H
    assert B == 1 and sum(OUT_CHUNKS) == S and DH == 20
    hbm = pl.BlockSpec(memory_space=pl.ANY)
    return pl.pallas_call(
        functools.partial(_kernel, S=S, D=D, DH=DH),
        out_shape=jax.ShapeDtypeStruct((B, S, D), A_x.dtype),
        in_specs=[hbm] * 8,
        out_specs=hbm,
        scratch_shapes=[
            pltpu.VMEM((S, D), BF16),
            pltpu.VMEM((3, D, D), BF16),
            pltpu.VMEM((D, D), BF16),
            pltpu.VMEM((D, F), BF16),
            pltpu.VMEM((F, D), BF16),
            pltpu.VMEM((S, D), BF16),
            pltpu.VMEM((D, S), F32),
            pltpu.VMEM((H // 2, S // 2, LANES), U32),
            pltpu.VMEM((H, 24, S), F32),
            pltpu.VMEM((D, S), F32),
            pltpu.VMEM((S, D), F32),
            pltpu.VMEM((2 * DH, (S // KC + XT) * VR, LANES), F32),
            pltpu.VMEM((2 * DH, 8, S), F32),
            pltpu.VMEM((H, 16, S), U32),
            pltpu.VMEM((8, D), F32),
            pltpu.VMEM((D, LANES), F32),
            pltpu.VMEM((F,), BF16),
            pltpu.VMEM((D,), BF16),
            pltpu.VMEM((D,), BF16),
            pltpu.SemaphoreType.DMA((9,)),
            pltpu.SemaphoreType.DMA((S // RC,)),
            pltpu.SemaphoreType.DMA((len(OUT_CHUNKS),)),
        ],
        compiler_params=pltpu.CompilerParams(vmem_limit_bytes=100 * 1024 * 1024),
    )(A_x, A_wqkv, A_wo, B_w1, B_b1, B_w2, B_b2, gate_w)
```

```python
import functools
import math

import jax
import jax.numpy as jnp
from jax import lax
import jax.experimental.pallas as pl
import jax.experimental.pallas.tpu as pltpu

H = 32
LANES = 128
TQ = 512
KC = 128
VR = 16
XT = 2
LAG = 2
SA = 2
DC = 4
RC = 512
TS = 256
F1A = 512
NLH = 32
OUT_CHUNKS = (512, 512, 512, 256, 128, 128)
SAFE_LOG2 = 40.0

NN = (((1,), (0,)), ((), ()))
F32 = jnp.float32
BF16 = jnp.bfloat16
U32 = jnp.uint32


def _kernel(x_hbm, wqkv_hbm, wo_hbm, w1_hbm, b1_hbm, w2_hbm, b2_hbm, gw_hbm,
            o_hbm,
            x_ref, wqkv_ref, wo_ref, w1_ref, w2_ref, o_ref,
            qt_ref, k_ref, vt_ref, ot_ref, fb_ref, kb_ref, qb_ref, qw_ref,
            mk_ref, mq_ref, b1_ref, b2_ref, gw_ref, in_sem, x_sem, out_sem, *, S, D, DH):
    NG = D // LANES
    NQ = S // TQ
    NKC = S // KC
    NR = S // RC
    NP = H // 2
    PW = 2 * DH
    FC = S // NP
    NJ = TQ // LANES
    FF = w1_ref.shape[1]
    KH = KC // 2
    qscale = (DH ** -0.5) * math.log2(math.e)
    xtiles = [(e + 1) * NKC // XT - 1 for e in range(XT)]
    assert 2 * NJ * XT == NKC

    def chunk(r, n=RC):
        return pl.ds(pl.multiple_of(r * n, n), n)

    def wcopy(n):
        return pltpu.make_async_copy(wqkv_hbm.at[:, pl.ds(n * D, D)], wqkv_ref.at[n], in_sem.at[n])

    def xcopy(r):
        return pltpu.make_async_copy(x_hbm.at[0, chunk(r), :], x_ref.at[chunk(r), :], x_sem.at[r])

    cp_wq, cp_wk, cp_wv = wcopy(0), wcopy(1), wcopy(2)
    cp_late = [pltpu.make_async_copy(a, b, in_sem.at[3 + n]) for n, (a, b) in enumerate((
        (w1_hbm, w1_ref), (w2_hbm, w2_ref), (wo_hbm, wo_ref),
        (b1_hbm, b1_ref), (b2_hbm, b2_ref), (gw_hbm, gw_ref)))]
    xcopy(0).start()
    cp_wk.start()
    mk_ref[...] = jnp.zeros(mk_ref.shape, F32)
    mq_ref[...] = jnp.zeros(mq_ref.shape, F32)

    def prep(pair, never, pace, n_pace):
        src = jnp.concatenate(
            [k_ref[pair, c * KH:c * KH + VR // 2, :] for c in range(NKC)]
            + [k_ref[pair, c * KH + VR // 2:c * KH + VR, :] for c in xtiles], axis=0)
        kpace = []
        for d in range(PW):
            kb = jnp.broadcast_to(src[:, d:d + 1], src.shape)
            kb_ref[d] = pltpu.bitcast(kb, BF16).astype(F32)
            kpace.append(kb[0:8])
        base = pl.multiple_of(PW * pair, 8)
        nt = (PW // 8) * (S // LANES)
        n = 0
        for t in range(PW // 8):
            for j in range(S // LANES):
                win = qt_ref[pl.ds(base + 8 * t, 8), j * LANES:(j + 1) * LANES]
                if n < n_pace:
                    after = pace[n * len(pace) // n_pace]
                else:
                    after = kpace[(n - n_pace) * PW // (nt - n_pace)]
                win = jnp.where(never, pltpu.bitcast(after, F32), win)
                n += 1
                qb_ref[8 * t:8 * t + 8, :, j * LANES:(j + 1) * LANES] = jnp.stack(
                    [jnp.broadcast_to(win[r:r + 1, :], (8, LANES)) for r in range(8)])

    def lane_fold_absmax(a):
        a = jnp.abs(a)
        out = a[:, 0:LANES]
        for j in range(1, a.shape[1] // LANES):
            out = jnp.maximum(out, a[:, j * LANES:(j + 1) * LANES])
        return out

    cp_wk.wait()
    for cp in [xcopy(r) for r in range(1, NR)] + [cp_wq, cp_wv]:
        cp.start()

    def proj_k(r, c):
        xcopy(r).wait()
        lane = lax.broadcasted_iota(jnp.int32, (RC // 2, LANES), 1)
        mk = mk_ref[...]
        k = jnp.dot(x_ref[chunk(r), :], wqkv_ref[1], preferred_element_type=F32)
        kp = pltpu.bitcast(k.astype(BF16), U32)
        grp = [kp[:, g * LANES:(g + 1) * LANES] for g in range(NG)]
        for p in range(NP):
            g, off = divmod(PW * p, LANES)
            t = grp[g]
            if off + PW > LANES:
                t = jnp.where(lane >= off, t, grp[g + 1])
            if off:
                t = pltpu.roll(t, LANES - off, 1)
            k_ref[p, chunk(r, RC // 2), :] = t
        mk_ref[...] = jnp.maximum(mk, jnp.max(jnp.abs(k).reshape(RC // 8, 8, D), axis=0))
        return c

    lax.fori_loop(0, NR, proj_k, 0)
    for cp in cp_late:
        cp.start()
    cp_wq.wait()
    cp_wv.wait()

    row24 = lax.broadcasted_iota(jnp.int32, (24, RC), 0)

    def proj_qv(r, mv, pace=None):
        rows = chunk(r)
        xc = x_ref[rows, :]
        qs, vs = [], []
        for j0 in range(0, D, LANES):
            q = jnp.dot(xc, wqkv_ref[0, :, j0:j0 + LANES], preferred_element_type=F32)
            qs.append((q * qscale).astype(BF16).astype(F32).T)
        for j0 in range(0, D, LANES):
            v = jnp.dot(xc, wqkv_ref[2, :, j0:j0 + LANES], preferred_element_type=F32)
            vs.append(v.astype(BF16).astype(F32).T)
            if pace is not None and j0 < D - LANES:
                pace += [v[r_:r_ + 8] for r_ in range(0, RC, 8)]
        qT = jnp.concatenate(qs, axis=0)
        vT = jnp.concatenate(vs, axis=0)
        qt_ref[:, rows] = qT
        zero8 = jnp.zeros((8, RC), F32)
        for h in range(H):
            odd = h % 2
            off = PW * (h // 2) + 16 * odd
            valid = (row24 >= 4) if odd else (row24 < DH)
            w = jnp.concatenate([jnp.where(valid, qT[off:off + 24, :], 0.0), zero8], axis=0)
            qw_ref[h, :, rows] = pltpu.bitcast(w.astype(BF16), U32)
            vt_ref[h, :, rows] = jnp.where(valid, vT[off:off + 24, :], 1.0)
        mq_ref[...] = jnp.maximum(mq_ref[...], lane_fold_absmax(qT))
        return jnp.maximum(mv, jnp.max(lane_fold_absmax(vT).reshape(D // 8, 8, LANES), axis=0))

    mv = lax.fori_loop(0, NR - 1, proj_qv, jnp.zeros((8, LANES), F32))
    for cp in cp_late:
        cp.wait()
    never0 = mv < 0.0
    pace0 = []
    mv = proj_qv(NR - 1, mv, pace0)
    prep(0, never0, pace0, (PW // 8) * (S // LANES))

    mk = jnp.max(mk_ref[...], axis=0, keepdims=True)
    col = lax.broadcasted_iota(jnp.int32, (H, D), 1)
    hrow = lax.broadcasted_iota(jnp.int32, (H, D), 0) * DH
    sel = jnp.where((col >= hrow) & (col < hrow + DH), mk, 0.0)
    bnd = jnp.dot(sel, mq_ref[...], preferred_element_type=F32)
    bnd = jnp.max(bnd.reshape(H // 8, 8, LANES), axis=0)
    vmax = jnp.max(mv)
    safe = (jnp.max(bnd) <= SAFE_LOG2) & (vmax <= 2.0 ** 60) & (vmax >= 2.0 ** -60)

    def ffn1(rows, c0, c1):
        b1 = b1_ref[...].astype(F32).reshape(1, -1)
        hh = jnp.dot(x_ref[rows, :], w1_ref[:, c0:c1], preferred_element_type=F32) + b1[:, c0:c1]
        hh = jnp.maximum(hh, 0.0)
        return pltpu.bitcast((hh * hh).astype(BF16), U32)

    def ffn2(rows, hh):
        b2 = b2_ref[...].astype(F32).reshape(1, -1)
        fb_ref[rows, :] = jnp.dot(pltpu.bitcast(hh, BF16), w2_ref[...], preferred_element_type=F32) + b2

    def scores_mxu(kc, h, odd, cols, width):
        w = qw_ref[h, :, cols]
        if odd:
            w = jnp.concatenate([jnp.zeros((8, width), U32), w], axis=0)
        w = pltpu.bitcast(w, BF16)
        return lax.dot_general(pltpu.bitcast(kc, BF16)[:, 0:w.shape[0]], w, NN, preferred_element_type=F32)

    def store_o(acc, pair, odd, cols):
        l = acc[0:1] if odd else acc[23:24]
        o = acc * (1.0 / l)
        base = pl.multiple_of(PW * pair, 8)
        if not odd:
            ot_ref[pl.ds(base, 24), cols] = o
        else:
            row8 = lax.broadcasted_iota(jnp.int32, (8, acc.shape[1]), 0)
            off = pl.multiple_of(base + 16, 8)
            old = ot_ref[pl.ds(off, 8), cols]
            ot_ref[pl.ds(off, 8), cols] = jnp.where(row8 >= 4, o[0:8], old)
            ot_ref[pl.ds(off + 8, 16), cols] = o[8:24]

    @pl.when(safe)
    def _fast():
        never = bnd < 0.0
        bnd_acc = jnp.tile(bnd, (3, NJ))
        never_acc = bnd_acc < 0.0

        def after(x, dep):
            n = dep.shape[0]
            x0 = jnp.where(never[None], dep, x[0:n])
            return x0 if n == x.shape[0] else jnp.concatenate([x0, x[n:]], axis=0)

        def scores_vpu(kb, qb, start=None, mid=None):
            acc = None
            for m, d in enumerate(range(0, DH, DC)):
                t = kb[d:d + DC] * qb[d:d + DC]
                if acc is not None:
                    if m == 2 and mid is not None:
                        acc = after(acc, mid)
                    t = jnp.concatenate([acc[None], t], axis=0)
                elif start is not None:
                    t = jnp.concatenate([after(t[0], start)[None], t[1:]], axis=0)
                acc = jnp.sum(t, axis=0)
            return acc

        def p_vpu(odd, qt, c, extra):
            dims = slice(odd * DH, (odd + 1) * DH)
            qb = qb_ref[dims, :, qt * TQ:(qt + 1) * TQ][:, None]
            qb = [qb[..., j * LANES:(j + 1) * LANES] for j in range(NJ)]
            e, pos = divmod(c, 2 * NJ)
            r0 = (NKC + e) * VR + 8 * (pos % 2)
            side = scores_vpu(kb_ref[dims, r0:r0 + 8, :][:, None], qb[pos // 2])
            extra.append(jnp.exp2(side[0]))
            kb = kb_ref[dims, c * VR:(c + 1) * VR, :].reshape(DH, VR // 8, 8, LANES)
            cols = []
            for j in range(NJ):
                cols.append(scores_vpu(kb, qb[j], cols[-1] if cols else None, side if j == NJ - 1 else None))
            parts = [jnp.exp2(jnp.concatenate([a.reshape(VR, LANES) for a in cols], axis=1))]
            if c in xtiles:
                parts.append(jnp.concatenate(
                    [jnp.concatenate(extra[0::2], axis=1), jnp.concatenate(extra[1::2], axis=1)], axis=0))
                extra.clear()
            return parts

        def p_mxu(i, odd, qt, c, blocks):
            b0 = min(blocks)
            kc = k_ref[i, c * KH + 8 * b0:c * KH + 8 * (b0 + len(blocks)), :]
            kc = jnp.concatenate([kc[8 * (b - b0):8 * (b - b0) + 8] for b in blocks], axis=0)
            sm = jnp.exp2(scores_mxu(kc, 2 * i + odd, odd, slice(qt * TQ, (qt + 1) * TQ), TQ))
            return {b: sm[16 * n:16 * n + 16] for n, b in enumerate(blocks)}

        def body(i, carry):
            T = 2 * NQ * NKC
            rows = chunk(i, FC)
            ps = {}
            extra = []
            acc = bnd_acc
            for t in range(T + LAG):
                if t < T:
                    u, c = divmod(t, NKC)
                    odd, qt = divmod(u, NQ)
                    parts = p_vpu(odd, qt, c, extra)
                    blocks = list(range(KC // 16 - 1, len(parts) - 1, -1))
                    res = p_mxu(i, odd, qt, c, blocks[:SA])
                if t == T:
                    hh = ffn1(rows, 0, F1A)
                if t >= LAG:
                    ub, cb = divmod(t - LAG, NKC)
                    oddb, qtb = divmod(ub, NQ)
                    vt = vt_ref[2 * i + oddb, :, cb * KC:(cb + 1) * KC]
                    a = lax.dot_general(vt, ps.pop(t - LAG).astype(BF16), NN, preferred_element_type=F32)
                    acc = jnp.where(never_acc, acc, a) if cb == 0 else acc + a
                    if cb == NKC - 1:
                        store_o(acc, i, oddb, slice(qtb * TQ, (qtb + 1) * TQ))
                if t < T:
                    res.update(p_mxu(i, odd, qt, c, blocks[SA:]))
                    ps[t] = jnp.concatenate(parts + [res[b] for b in sorted(res)], axis=0)
            hh = jnp.concatenate([hh, ffn1(rows, F1A, FF)], axis=1)
            ffn2(rows, hh)
            pace = [hh[r:r + 8, c:c + LANES] for c in range(F1A, FF, LANES) for r in range(0, FC // 2, 8)]
            prep(jnp.minimum(i + 1, NP - 1), never, pace, NLH)
            return carry

        lax.fori_loop(0, NP, body, 0)

    @pl.when(jnp.logical_not(safe))
    def _fallback():
        def unit(u, carry):
            i = u // (S // TS)
            cols = chunk(u % (S // TS), TS)
            for odd in range(2):
                s = scores_mxu(k_ref[i], 2 * i + odd, odd, cols, TS)
                m = jnp.max(s, axis=0, keepdims=True)
                p = jnp.exp2(s - m).astype(BF16)
                acc = lax.dot_general(vt_ref[2 * i + odd], p, NN, preferred_element_type=F32)
                store_o(acc, i, odd, cols)
            return carry

        lax.fori_loop(0, NP * (S // TS), unit, 0)

        def ffn(i, carry):
            rows = chunk(i, 64)
            ffn2(rows, ffn1(rows, 0, FF))
            return carry

        lax.fori_loop(0, S // 64, ffn, 0)

    gw = gw_ref[...].astype(F32).reshape(1, -1)
    copies = []
    r0 = 0
    for n, sz in enumerate(OUT_CHUNKS):
        rows = pl.ds(r0, sz)
        r0 += sz
        o = ot_ref[:, rows].T.astype(BF16)
        a = jnp.dot(o, wo_ref[...], preferred_element_type=F32)
        z = jnp.sum(x_ref[rows, :].astype(F32) * gw, axis=-1, keepdims=True)
        g = 1.0 / (1.0 + jnp.exp(-z))
        o_ref[rows, :] = (g * a + (1.0 - g) * fb_ref[rows, :]).astype(o_ref.dtype)
        cp = pltpu.make_async_copy(o_ref.at[rows, :], o_hbm.at[0, rows, :], out_sem.at[n])
        cp.start()
        copies.append(cp)
    for cp in copies:
        cp.wait()


@jax.jit
def pallas_gated_mix__softmax_full_mha__dense_activation_squared_relu__prompt_kernel(
    A_x: jax.Array,
    A_wqkv: jax.Array,
    A_wo: jax.Array,
    B_x: jax.Array,
    B_w1: jax.Array,
    B_b1: jax.Array,
    B_w2: jax.Array,
    B_b2: jax.Array,
    gate_w: jax.Array,
):
    del B_x
    B, S, D = A_x.shape
    F = B_w1.shape[1]
    DH = D // H
    assert B == 1 and sum(OUT_CHUNKS) == S and DH == 20
    hbm = pl.BlockSpec(memory_space=pl.ANY)
    return pl.pallas_call(
        functools.partial(_kernel, S=S, D=D, DH=DH),
        out_shape=jax.ShapeDtypeStruct((B, S, D), A_x.dtype),
        in_specs=[hbm] * 8,
        out_specs=hbm,
        scratch_shapes=[
            pltpu.VMEM((S, D), BF16),
            pltpu.VMEM((3, D, D), BF16),
            pltpu.VMEM((D, D), BF16),
            pltpu.VMEM((D, F), BF16),
            pltpu.VMEM((F, D), BF16),
            pltpu.VMEM((S, D), BF16),
            pltpu.VMEM((D, S), F32),
            pltpu.VMEM((H // 2, S // 2, LANES), U32),
            pltpu.VMEM((H, 24, S), F32),
            pltpu.VMEM((D, S), F32),
            pltpu.VMEM((S, D), F32),
            pltpu.VMEM((2 * DH, (S // KC + XT) * VR, LANES), F32),
            pltpu.VMEM((2 * DH, 8, S), F32),
            pltpu.VMEM((H, 16, S), U32),
            pltpu.VMEM((8, D), F32),
            pltpu.VMEM((D, LANES), F32),
            pltpu.VMEM((F,), BF16),
            pltpu.VMEM((D,), BF16),
            pltpu.VMEM((D,), BF16),
            pltpu.SemaphoreType.DMA((9,)),
            pltpu.SemaphoreType.DMA((S // RC,)),
            pltpu.SemaphoreType.DMA((len(OUT_CHUNKS),)),
        ],
        compiler_params=pltpu.CompilerParams(vmem_limit_bytes=100 * 1024 * 1024),
    )(A_x, A_wqkv, A_wo, B_w1, B_b1, B_w2, B_b2, gate_w)
```

```python
import functools
import math

import jax
import jax.numpy as jnp
from jax import lax
import jax.experimental.pallas as pl
import jax.experimental.pallas.tpu as pltpu

H = 32
LANES = 128
TQ = 512
KC = 128
VR = 16
XT = 2
LAG = 2
SA = 2
DC = 4
RC = 512
TS = 256
F1A = 512
NLH = 32
K0 = 320
NK = 2
OUT_CHUNKS = (512, 512, 512, 256, 128, 128)
SAFE_LOG2 = 40.0

NN = (((1,), (0,)), ((), ()))
F32 = jnp.float32
BF16 = jnp.bfloat16
U32 = jnp.uint32


def _kernel(x_hbm, wqkv_hbm, wo_hbm, w1_hbm, b1_hbm, w2_hbm, b2_hbm, gw_hbm,
            o_hbm,
            x_ref, wqkv_ref, wo_ref, w1_ref, w2_ref, o_ref,
            qt_ref, k_ref, vt_ref, ot_ref, fb_ref, kb_ref, qb_ref, qw_ref,
            mk_ref, mq_ref, b1_ref, b2_ref, gw_ref, in_sem, x_sem, out_sem, *, S, D, DH):
    NG = D // LANES
    NQ = S // TQ
    NKC = S // KC
    NR = S // RC
    NP = H // 2
    PW = 2 * DH
    FC = S // NP
    NJ = TQ // LANES
    FF = w1_ref.shape[1]
    KH = KC // 2
    qscale = (DH ** -0.5) * math.log2(math.e)
    xtiles = [(e + 1) * NKC // XT - 1 for e in range(XT)]
    assert 2 * NJ * XT == NKC

    def chunk(r, n=RC):
        return pl.ds(pl.multiple_of(r * n, n), n)

    def wcopy(n):
        return pltpu.make_async_copy(wqkv_hbm.at[:, pl.ds(n * D, D)], wqkv_ref.at[n], in_sem.at[n])

    KR = (S - K0) // NK
    assert KR * NK + K0 == S and KR % 16 == 0

    def krows(r, div=1):
        if isinstance(r, int) and r < 0:
            return pl.ds(0, K0 // div)
        return pl.ds(pl.multiple_of(K0 // div + r * (KR // div), 16 // div), KR // div)

    def xcopy(r):
        return pltpu.make_async_copy(x_hbm.at[0, krows(r), :], x_ref.at[krows(r), :], x_sem.at[r + 1])

    cp_wq, cp_wk, cp_wv = wcopy(0), wcopy(1), wcopy(2)
    cp_late = [pltpu.make_async_copy(a, b, in_sem.at[3 + n]) for n, (a, b) in enumerate((
        (w1_hbm, w1_ref), (w2_hbm, w2_ref), (wo_hbm, wo_ref),
        (b1_hbm, b1_ref), (b2_hbm, b2_ref), (gw_hbm, gw_ref)))]
    xcopy(-1).start()
    cp_wk.start()
    mk_ref[...] = jnp.zeros(mk_ref.shape, F32)
    mq_ref[...] = jnp.zeros(mq_ref.shape, F32)

    def prep(pair, never, pace, n_pace):
        src = jnp.concatenate(
            [k_ref[pair, c * KH:c * KH + VR // 2, :] for c in range(NKC)]
            + [k_ref[pair, c * KH + VR // 2:c * KH + VR, :] for c in xtiles], axis=0)
        kpace = []
        for d in range(PW):
            kb = jnp.broadcast_to(src[:, d:d + 1], src.shape)
            kb_ref[d] = pltpu.bitcast(kb, BF16).astype(F32)
            kpace.append(kb[0:8])
        base = pl.multiple_of(PW * pair, 8)
        nt = (PW // 8) * (S // LANES)
        n = 0
        for t in range(PW // 8):
            for j in range(S // LANES):
                win = qt_ref[pl.ds(base + 8 * t, 8), j * LANES:(j + 1) * LANES]
                if n < n_pace:
                    after = pace[n * len(pace) // n_pace]
                else:
                    after = kpace[(n - n_pace) * PW // (nt - n_pace)]
                win = jnp.where(never, pltpu.bitcast(after, F32), win)
                n += 1
                qb_ref[8 * t:8 * t + 8, :, j * LANES:(j + 1) * LANES] = jnp.stack(
                    [jnp.broadcast_to(win[r:r + 1, :], (8, LANES)) for r in range(8)])

    def lane_fold_absmax(a):
        a = jnp.abs(a)
        out = a[:, 0:LANES]
        for j in range(1, a.shape[1] // LANES):
            out = jnp.maximum(out, a[:, j * LANES:(j + 1) * LANES])
        return out

    xcopy(-1).wait()
    xcopy(0).start()
    cp_wk.wait()
    for cp in [xcopy(r) for r in range(1, NK)] + [cp_wq, cp_wv]:
        cp.start()

    def proj_k(r, c):
        first = isinstance(r, int)
        n = K0 if first else KR
        if not first:
            xcopy(r).wait()
        lane = lax.broadcasted_iota(jnp.int32, (n // 2, LANES), 1)
        mk = mk_ref[...]
        k = jnp.dot(x_ref[krows(r), :], wqkv_ref[1], preferred_element_type=F32)
        kp = pltpu.bitcast(k.astype(BF16), U32)
        grp = [kp[:, g * LANES:(g + 1) * LANES] for g in range(NG)]
        for p in range(NP):
            g, off = divmod(PW * p, LANES)
            t = grp[g]
            if off + PW > LANES:
                t = jnp.where(lane >= off, t, grp[g + 1])
            if off:
                t = pltpu.roll(t, LANES - off, 1)
            k_ref[p, krows(r, 2), :] = t
        mk_ref[...] = jnp.maximum(mk, jnp.max(jnp.abs(k).reshape(n // 8, 8, D), axis=0))
        return c

    proj_k(-1, 0)
    lax.fori_loop(0, NK, proj_k, 0)
    for cp in cp_late:
        cp.start()
    cp_wq.wait()
    cp_wv.wait()

    row24 = lax.broadcasted_iota(jnp.int32, (24, RC), 0)

    def proj_qv(r, mv, pace=None):
        rows = chunk(r)
        xc = x_ref[rows, :]
        qs, vs = [], []
        for j0 in range(0, D, LANES):
            q = jnp.dot(xc, wqkv_ref[0, :, j0:j0 + LANES], preferred_element_type=F32)
            qs.append((q * qscale).astype(BF16).astype(F32).T)
        for j0 in range(0, D, LANES):
            v = jnp.dot(xc, wqkv_ref[2, :, j0:j0 + LANES], preferred_element_type=F32)
            vs.append(v.astype(BF16).astype(F32).T)
            if pace is not None and j0 < D - LANES:
                pace += [v[r_:r_ + 8] for r_ in range(0, RC, 8)]
        qT = jnp.concatenate(qs, axis=0)
        vT = jnp.concatenate(vs, axis=0)
        qt_ref[:, rows] = qT
        zero8 = jnp.zeros((8, RC), F32)
        for h in range(H):
            odd = h % 2
            off = PW * (h // 2) + 16 * odd
            valid = (row24 >= 4) if odd else (row24 < DH)
            w = jnp.concatenate([jnp.where(valid, qT[off:off + 24, :], 0.0), zero8], axis=0)
            qw_ref[h, :, rows] = pltpu.bitcast(w.astype(BF16), U32)
            vt_ref[h, :, rows] = jnp.where(valid, vT[off:off + 24, :], 1.0)
        mq_ref[...] = jnp.maximum(mq_ref[...], lane_fold_absmax(qT))
        return jnp.maximum(mv, jnp.max(lane_fold_absmax(vT).reshape(D // 8, 8, LANES), axis=0))

    mv = lax.fori_loop(0, NR - 1, proj_qv, jnp.zeros((8, LANES), F32))
    for cp in cp_late:
        cp.wait()
    never0 = mv < 0.0
    pace0 = []
    mv = proj_qv(NR - 1, mv, pace0)
    prep(0, never0, pace0, (PW // 8) * (S // LANES))

    mk = jnp.max(mk_ref[...], axis=0, keepdims=True)
    col = lax.broadcasted_iota(jnp.int32, (H, D), 1)
    hrow = lax.broadcasted_iota(jnp.int32, (H, D), 0) * DH
    sel = jnp.where((col >= hrow) & (col < hrow + DH), mk, 0.0)
    bnd = jnp.dot(sel, mq_ref[...], preferred_element_type=F32)
    bnd = jnp.max(bnd.reshape(H // 8, 8, LANES), axis=0)
    vmax = jnp.max(mv)
    safe = (jnp.max(bnd) <= SAFE_LOG2) & (vmax <= 2.0 ** 60) & (vmax >= 2.0 ** -60)

    def ffn1(rows, c0, c1):
        b1 = b1_ref[...].astype(F32).reshape(1, -1)
        hh = jnp.dot(x_ref[rows, :], w1_ref[:, c0:c1], preferred_element_type=F32) + b1[:, c0:c1]
        hh = jnp.maximum(hh, 0.0)
        return pltpu.bitcast((hh * hh).astype(BF16), U32)

    def ffn2(rows, hh):
        b2 = b2_ref[...].astype(F32).reshape(1, -1)
        fb_ref[rows, :] = jnp.dot(pltpu.bitcast(hh, BF16), w2_ref[...], preferred_element_type=F32) + b2

    def scores_mxu(kc, h, odd, cols, width):
        w = qw_ref[h, :, cols]
        if odd:
            w = jnp.concatenate([jnp.zeros((8, width), U32), w], axis=0)
        w = pltpu.bitcast(w, BF16)
        return lax.dot_general(pltpu.bitcast(kc, BF16)[:, 0:w.shape[0]], w, NN, preferred_element_type=F32)

    def store_o(acc, pair, odd, cols):
        l = acc[0:1] if odd else acc[23:24]
        o = acc * (1.0 / l)
        base = pl.multiple_of(PW * pair, 8)
        if not odd:
            ot_ref[pl.ds(base, 24), cols] = o
        else:
            row8 = lax.broadcasted_iota(jnp.int32, (8, acc.shape[1]), 0)
            off = pl.multiple_of(base + 16, 8)
            old = ot_ref[pl.ds(off, 8), cols]
            ot_ref[pl.ds(off, 8), cols] = jnp.where(row8 >= 4, o[0:8], old)
            ot_ref[pl.ds(off + 8, 16), cols] = o[8:24]

    @pl.when(safe)
    def _fast():
        never = bnd < 0.0
        bnd_acc = jnp.tile(bnd, (3, NJ))
        never_acc = bnd_acc < 0.0

        def after(x, dep):
            n = dep.shape[0]
            x0 = jnp.where(never[None], dep, x[0:n])
            return x0 if n == x.shape[0] else jnp.concatenate([x0, x[n:]], axis=0)

        def scores_vpu(kb, qb, start=None, mid=None):
            acc = None
            for m, d in enumerate(range(0, DH, DC)):
                t = kb[d:d + DC] * qb[d:d + DC]
                if acc is not None:
                    if m == 2 and mid is not None:
                        acc = after(acc, mid)
                    t = jnp.concatenate([acc[None], t], axis=0)
                elif start is not None:
                    t = jnp.concatenate([after(t[0], start)[None], t[1:]], axis=0)
                acc = jnp.sum(t, axis=0)
            return acc

        def p_vpu(odd, qt, c, extra):
            dims = slice(odd * DH, (odd + 1) * DH)
            qb = qb_ref[dims, :, qt * TQ:(qt + 1) * TQ][:, None]
            qb = [qb[..., j * LANES:(j + 1) * LANES] for j in range(NJ)]
            e, pos = divmod(c, 2 * NJ)
            r0 = (NKC + e) * VR + 8 * (pos % 2)
            side = scores_vpu(kb_ref[dims, r0:r0 + 8, :][:, None], qb[pos // 2])
            extra.append(jnp.exp2(side[0]))
            kb = kb_ref[dims, c * VR:(c + 1) * VR, :].reshape(DH, VR // 8, 8, LANES)
            cols = []
            for j in range(NJ):
                cols.append(scores_vpu(kb, qb[j], cols[-1] if cols else None, side if j == NJ - 1 else None))
            parts = [jnp.exp2(jnp.concatenate([a.reshape(VR, LANES) for a in cols], axis=1))]
            if c in xtiles:
                parts.append(jnp.concatenate(
                    [jnp.concatenate(extra[0::2], axis=1), jnp.concatenate(extra[1::2], axis=1)], axis=0))
                extra.clear()
            return parts

        def p_mxu(i, odd, qt, c, blocks):
            b0 = min(blocks)
            kc = k_ref[i, c * KH + 8 * b0:c * KH + 8 * (b0 + len(blocks)), :]
            kc = jnp.concatenate([kc[8 * (b - b0):8 * (b - b0) + 8] for b in blocks], axis=0)
            sm = jnp.exp2(scores_mxu(kc, 2 * i + odd, odd, slice(qt * TQ, (qt + 1) * TQ), TQ))
            return {b: sm[16 * n:16 * n + 16] for n, b in enumerate(blocks)}

        def body(i, carry):
            T = 2 * NQ * NKC
            rows = chunk(i, FC)
            ps = {}
            extra = []
            acc = bnd_acc
            for t in range(T + LAG):
                if t < T:
                    u, c = divmod(t, NKC)
                    odd, qt = divmod(u, NQ)
                    parts = p_vpu(odd, qt, c, extra)
                    blocks = list(range(KC // 16 - 1, len(parts) - 1, -1))
                    res = p_mxu(i, odd, qt, c, blocks[:SA])
                if t == T:
                    hh = ffn1(rows, 0, F1A)
                if t >= LAG:
                    ub, cb = divmod(t - LAG, NKC)
                    oddb, qtb = divmod(ub, NQ)
                    vt = vt_ref[2 * i + oddb, :, cb * KC:(cb + 1) * KC]
                    a = lax.dot_general(vt, ps.pop(t - LAG).astype(BF16), NN, preferred_element_type=F32)
                    acc = jnp.where(never_acc, acc, a) if cb == 0 else acc + a
                    if cb == NKC - 1:
                        store_o(acc, i, oddb, slice(qtb * TQ, (qtb + 1) * TQ))
                if t < T:
                    res.update(p_mxu(i, odd, qt, c, blocks[SA:]))
                    ps[t] = jnp.concatenate(parts + [res[b] for b in sorted(res)], axis=0)
            hh = jnp.concatenate([hh, ffn1(rows, F1A, FF)], axis=1)
            ffn2(rows, hh)
            pace = [hh[r:r + 8, c:c + LANES] for c in range(F1A, FF, LANES) for r in range(0, FC // 2, 8)]
            prep(jnp.minimum(i + 1, NP - 1), never, pace, NLH)
            return carry

        lax.fori_loop(0, NP, body, 0)

    @pl.when(jnp.logical_not(safe))
    def _fallback():
        def unit(u, carry):
            i = u // (S // TS)
            cols = chunk(u % (S // TS), TS)
            for odd in range(2):
                s = scores_mxu(k_ref[i], 2 * i + odd, odd, cols, TS)
                m = jnp.max(s, axis=0, keepdims=True)
                p = jnp.exp2(s - m).astype(BF16)
                acc = lax.dot_general(vt_ref[2 * i + odd], p, NN, preferred_element_type=F32)
                store_o(acc, i, odd, cols)
            return carry

        lax.fori_loop(0, NP * (S // TS), unit, 0)

        def ffn(i, carry):
            rows = chunk(i, 64)
            ffn2(rows, ffn1(rows, 0, FF))
            return carry

        lax.fori_loop(0, S // 64, ffn, 0)

    gw = gw_ref[...].astype(F32).reshape(1, -1)
    copies = []
    r0 = 0
    for n, sz in enumerate(OUT_CHUNKS):
        rows = pl.ds(r0, sz)
        r0 += sz
        o = ot_ref[:, rows].T.astype(BF16)
        a = jnp.dot(o, wo_ref[...], preferred_element_type=F32)
        z = jnp.sum(x_ref[rows, :].astype(F32) * gw, axis=-1, keepdims=True)
        g = 1.0 / (1.0 + jnp.exp(-z))
        o_ref[rows, :] = (g * a + (1.0 - g) * fb_ref[rows, :]).astype(o_ref.dtype)
        cp = pltpu.make_async_copy(o_ref.at[rows, :], o_hbm.at[0, rows, :], out_sem.at[n])
        cp.start()
        copies.append(cp)
    for cp in copies:
        cp.wait()


@jax.jit
def pallas_gated_mix__softmax_full_mha__dense_activation_squared_relu__prompt_kernel(
    A_x: jax.Array,
    A_wqkv: jax.Array,
    A_wo: jax.Array,
    B_x: jax.Array,
    B_w1: jax.Array,
    B_b1: jax.Array,
    B_w2: jax.Array,
    B_b2: jax.Array,
    gate_w: jax.Array,
):
    del B_x
    B, S, D = A_x.shape
    F = B_w1.shape[1]
    DH = D // H
    assert B == 1 and sum(OUT_CHUNKS) == S and DH == 20
    hbm = pl.BlockSpec(memory_space=pl.ANY)
    return pl.pallas_call(
        functools.partial(_kernel, S=S, D=D, DH=DH),
        out_shape=jax.ShapeDtypeStruct((B, S, D), A_x.dtype),
        in_specs=[hbm] * 8,
        out_specs=hbm,
        scratch_shapes=[
            pltpu.VMEM((S, D), BF16),
            pltpu.VMEM((3, D, D), BF16),
            pltpu.VMEM((D, D), BF16),
            pltpu.VMEM((D, F), BF16),
            pltpu.VMEM((F, D), BF16),
            pltpu.VMEM((S, D), BF16),
            pltpu.VMEM((D, S), F32),
            pltpu.VMEM((H // 2, S // 2, LANES), U32),
            pltpu.VMEM((H, 24, S), F32),
            pltpu.VMEM((D, S), F32),
            pltpu.VMEM((S, D), F32),
            pltpu.VMEM((2 * DH, (S // KC + XT) * VR, LANES), F32),
            pltpu.VMEM((2 * DH, 8, S), F32),
            pltpu.VMEM((H, 16, S), U32),
            pltpu.VMEM((8, D), F32),
            pltpu.VMEM((D, LANES), F32),
            pltpu.VMEM((F,), BF16),
            pltpu.VMEM((D,), BF16),
            pltpu.VMEM((D,), BF16),
            pltpu.SemaphoreType.DMA((9,)),
            pltpu.SemaphoreType.DMA((NK + 1,)),
            pltpu.SemaphoreType.DMA((len(OUT_CHUNKS),)),
        ],
        compiler_params=pltpu.CompilerParams(vmem_limit_bytes=100 * 1024 * 1024),
    )(A_x, A_wqkv, A_wo, B_w1, B_b1, B_w2, B_b2, gate_w)
```

```python
import functools
import math

import jax
import jax.numpy as jnp
from jax import lax
import jax.experimental.pallas as pl
import jax.experimental.pallas.tpu as pltpu

H = 32
LANES = 128
TQ = 512
KC = 128
VR = 16
XT = 2
LAG = 2
SA = 2
DC = 4
RC = 512
TS = 256
F1A = 512
NLH = 32
K0 = 320
NK = 2
OUT_CHUNKS = (512, 512, 512, 256, 128, 128)
SAFE_LOG2 = 40.0

NN = (((1,), (0,)), ((), ()))
F32 = jnp.float32
BF16 = jnp.bfloat16
U32 = jnp.uint32


def _kernel(x_hbm, wqkv_hbm, wo_hbm, w1_hbm, b1_hbm, w2_hbm, b2_hbm, gw_hbm,
            o_hbm,
            x_ref, wqkv_ref, wo_ref, w1_ref, w2_ref, o_ref,
            qt_ref, k_ref, vt_ref, ot_ref, fb_ref, kb_ref, qb_ref, qw_ref,
            mk_ref, mq_ref, b1_ref, b2_ref, gw_ref, in_sem, x_sem, out_sem, *, S, D, DH):
    NG = D // LANES
    NQ = S // TQ
    NKC = S // KC
    NR = S // RC
    NP = H // 2
    PW = 2 * DH
    FC = S // NP
    NJ = TQ // LANES
    FF = w1_ref.shape[1]
    KH = KC // 2
    qscale = (DH ** -0.5) * math.log2(math.e)
    xtiles = [(e + 1) * NKC // XT - 1 for e in range(XT)]
    assert 2 * NJ * XT == NKC

    def chunk(r, n=RC):
        return pl.ds(pl.multiple_of(r * n, n), n)

    def wcopy(n):
        return pltpu.make_async_copy(wqkv_hbm.at[:, pl.ds(n * D, D)], wqkv_ref.at[n], in_sem.at[n])

    KR = (S - K0) // NK
    assert KR * NK + K0 == S and KR % 16 == 0

    def krows(r, div=1):
        if isinstance(r, int) and r < 0:
            return pl.ds(0, K0 // div)
        return pl.ds(pl.multiple_of(K0 // div + r * (KR // div), 16 // div), KR // div)

    def xcopy(r):
        return pltpu.make_async_copy(x_hbm.at[0, krows(r), :], x_ref.at[krows(r), :], x_sem.at[r + 1])

    cp_wq, cp_wk, cp_wv = wcopy(0), wcopy(1), wcopy(2)
    cp_late = [pltpu.make_async_copy(a, b, in_sem.at[3 + n]) for n, (a, b) in enumerate((
        (w1_hbm, w1_ref), (w2_hbm, w2_ref), (wo_hbm, wo_ref),
        (b1_hbm, b1_ref), (b2_hbm, b2_ref), (gw_hbm, gw_ref)))]
    xcopy(-1).start()
    cp_wk.start()
    mk_ref[...] = jnp.zeros(mk_ref.shape, F32)
    mq_ref[...] = jnp.zeros(mq_ref.shape, F32)

    def prep(pair, never, pace, n_pace):
        src = jnp.concatenate(
            [k_ref[pair, c * KH:c * KH + VR // 2, :] for c in range(NKC)]
            + [k_ref[pair, c * KH + VR // 2:c * KH + VR, :] for c in xtiles], axis=0)
        kpace = []
        for d in range(PW):
            kb = jnp.broadcast_to(src[:, d:d + 1], src.shape)
            kb_ref[d] = pltpu.bitcast(kb, BF16).astype(F32)
            kpace.append(kb[0:8])
        base = pl.multiple_of(PW * pair, 8)
        nt = (PW // 8) * (S // LANES)
        n = 0
        for t in range(PW // 8):
            for j in range(S // LANES):
                win = qt_ref[pl.ds(base + 8 * t, 8), j * LANES:(j + 1) * LANES]
                if n < n_pace:
                    after = pace[n * len(pace) // n_pace]
                else:
                    after = kpace[(n - n_pace) * PW // (nt - n_pace)]
                win = jnp.where(never, pltpu.bitcast(after, F32), win)
                n += 1
                qb_ref[8 * t:8 * t + 8, :, j * LANES:(j + 1) * LANES] = jnp.stack(
                    [jnp.broadcast_to(win[r:r + 1, :], (8, LANES)) for r in range(8)])

    def lane_fold_absmax(a):
        a = jnp.abs(a)
        out = a[:, 0:LANES]
        for j in range(1, a.shape[1] // LANES):
            out = jnp.maximum(out, a[:, j * LANES:(j + 1) * LANES])
        return out

    xcopy(-1).wait()
    xcopy(0).start()
    cp_wk.wait()
    for cp in [xcopy(r) for r in range(1, NK)] + [cp_wq, cp_wv]:
        cp.start()

    def proj_k(r, c):
        first = isinstance(r, int)
        n = K0 if first else KR
        if not first:
            xcopy(r).wait()
        lane = lax.broadcasted_iota(jnp.int32, (n // 2, LANES), 1)
        mk = mk_ref[...]
        k = jnp.dot(x_ref[krows(r), :], wqkv_ref[1], preferred_element_type=F32)
        kp = pltpu.bitcast(k.astype(BF16), U32)
        grp = [kp[:, g * LANES:(g + 1) * LANES] for g in range(NG)]
        for p in range(NP):
            g, off = divmod(PW * p, LANES)
            t = grp[g]
            if off + PW > LANES:
                t = jnp.where(lane >= off, t, grp[g + 1])
            if off:
                t = pltpu.roll(t, LANES - off, 1)
            k_ref[p, krows(r, 2), :] = t
        mk_ref[...] = jnp.maximum(mk, jnp.max(jnp.abs(k).reshape(n // 8, 8, D), axis=0))
        return c

    proj_k(-1, 0)
    lax.fori_loop(0, NK, proj_k, 0)
    for cp in cp_late:
        cp.start()
    cp_wq.wait()
    cp_wv.wait()

    row24 = lax.broadcasted_iota(jnp.int32, (24, RC), 0)

    def proj_qv(r, mv, pace=None):
        rows = chunk(r)
        xc = x_ref[rows, :]
        qs, vs = [], []
        for j0 in range(0, D, LANES):
            q = jnp.dot(xc, wqkv_ref[0, :, j0:j0 + LANES], preferred_element_type=F32)
            qs.append((q * qscale).astype(BF16).astype(F32).T)
        for j0 in range(0, D, LANES):
            v = jnp.dot(xc, wqkv_ref[2, :, j0:j0 + LANES], preferred_element_type=F32)
            vs.append(v.astype(BF16).astype(F32).T)
            if pace is not None and j0 < D - LANES:
                pace += [v[r_:r_ + 8] for r_ in range(0, RC, 8)]
        qT = jnp.concatenate(qs, axis=0)
        vT = jnp.concatenate(vs, axis=0)
        qt_ref[:, rows] = qT
        zero8 = jnp.zeros((8, RC), F32)
        for h in range(H):
            odd = h % 2
            off = PW * (h // 2) + 16 * odd
            valid = (row24 >= 4) if odd else (row24 < DH)
            w = jnp.concatenate([jnp.where(valid, qT[off:off + 24, :], 0.0), zero8], axis=0)
            qw_ref[h, :, rows] = pltpu.bitcast(w.astype(BF16), U32)
            vt_ref[h, :, rows] = jnp.where(valid, vT[off:off + 24, :], 1.0)
        mq_ref[...] = jnp.maximum(mq_ref[...], lane_fold_absmax(qT))
        return jnp.maximum(mv, jnp.max(lane_fold_absmax(vT).reshape(D // 8, 8, LANES), axis=0))

    mv = lax.fori_loop(0, NR - 1, proj_qv, jnp.zeros((8, LANES), F32))
    for cp in cp_late:
        cp.wait()
    never0 = mv < 0.0
    pace0 = []
    mv = proj_qv(NR - 1, mv, pace0)
    prep(0, never0, pace0, (PW // 8) * (S // LANES))

    mk = jnp.max(mk_ref[...], axis=0, keepdims=True)
    col = lax.broadcasted_iota(jnp.int32, (H, D), 1)
    hrow = lax.broadcasted_iota(jnp.int32, (H, D), 0) * DH
    sel = jnp.where((col >= hrow) & (col < hrow + DH), mk, 0.0)
    bnd = jnp.dot(sel, mq_ref[...], preferred_element_type=F32)
    bnd = jnp.max(bnd.reshape(H // 8, 8, LANES), axis=0)
    vmax = jnp.max(mv)
    safe = (jnp.max(bnd) <= SAFE_LOG2) & (vmax <= 2.0 ** 60) & (vmax >= 2.0 ** -60)

    def ffn1(rows, c0, c1):
        b1 = b1_ref[...].astype(F32).reshape(1, -1)
        hh = jnp.dot(x_ref[rows, :], w1_ref[:, c0:c1], preferred_element_type=F32) + b1[:, c0:c1]
        hh = jnp.maximum(hh, 0.0)
        return pltpu.bitcast((hh * hh).astype(BF16), U32)

    def ffn2(rows, hh):
        b2 = b2_ref[...].astype(F32).reshape(1, -1)
        fb_ref[rows, :] = jnp.dot(pltpu.bitcast(hh, BF16), w2_ref[...], preferred_element_type=F32) + b2

    def scores_mxu(kc, h, odd, cols, width):
        w = qw_ref[h, :, cols]
        if odd:
            w = jnp.concatenate([jnp.zeros((8, width), U32), w], axis=0)
        w = pltpu.bitcast(w, BF16)
        return lax.dot_general(pltpu.bitcast(kc, BF16)[:, 0:w.shape[0]], w, NN, preferred_element_type=F32)

    def store_o(acc, pair, odd, cols):
        l = acc[0:1] if odd else acc[23:24]
        o = acc * (1.0 / l)
        base = pl.multiple_of(PW * pair, 8)
        if not odd:
            ot_ref[pl.ds(base, 24), cols] = o
        else:
            row8 = lax.broadcasted_iota(jnp.int32, (8, acc.shape[1]), 0)
            off = pl.multiple_of(base + 16, 8)
            old = ot_ref[pl.ds(off, 8), cols]
            ot_ref[pl.ds(off, 8), cols] = jnp.where(row8 >= 4, o[0:8], old)
            ot_ref[pl.ds(off + 8, 16), cols] = o[8:24]

    @pl.when(safe)
    def _fast():
        never = bnd < 0.0
        bnd_acc = jnp.tile(bnd, (3, NJ))
        never_acc = bnd_acc < 0.0

        def after(x, dep):
            return jnp.where(never[None], dep, x)

        def scores_vpu(kb, qb, start):
            acc = None
            for d in range(0, DH, DC):
                t = kb[d:d + DC] * qb[d:d + DC]
                if acc is not None:
                    t = jnp.concatenate([acc[None], t], axis=0)
                elif start is not None:
                    t = jnp.concatenate([after(t[0], start)[None], t[1:]], axis=0)
                acc = jnp.sum(t, axis=0)
            return acc

        def p_vpu(odd, qt, c, extra):
            dims = slice(odd * DH, (odd + 1) * DH)
            qb = qb_ref[dims, :, qt * TQ:(qt + 1) * TQ][:, None]
            kb = kb_ref[dims, c * VR:(c + 1) * VR, :].reshape(DH, VR // 8, 8, LANES)
            e, pos = divmod(c, 2 * NJ)
            jx, rx = divmod(pos, 2)
            rest = [j for j in range(NJ) if j != jx]
            cols = {}
            prev = None
            for j in rest[:2] + [jx] + rest[2:]:
                q = qb[..., j * LANES:(j + 1) * LANES]
                if j == jx:
                    r0 = (NKC + e) * VR + 8 * rx
                    kx = kb_ref[dims, r0:r0 + 8, :][:, None]
                    w = scores_vpu(jnp.concatenate([kb, kx], axis=1), q,
                                   jnp.concatenate([prev, prev[1:2]], axis=0))
                    extra[(j, rx)] = jnp.exp2(w[2])
                    cols[j] = w[0:2]
                    prev = jnp.concatenate([w[0:1], after(w[1:2], w[2:3])], axis=0)
                else:
                    prev = cols[j] = scores_vpu(kb, q, prev)
            parts = [jnp.exp2(jnp.concatenate([cols[j].reshape(VR, LANES) for j in range(NJ)], axis=1))]
            if c in xtiles:
                parts.append(jnp.concatenate(
                    [jnp.concatenate([extra.pop((j, r)) for j in range(NJ)], axis=1) for r in range(2)], axis=0))
            return parts

        def p_mxu(i, odd, qt, c, blocks):
            b0 = min(blocks)
            kc = k_ref[i, c * KH + 8 * b0:c * KH + 8 * (b0 + len(blocks)), :]
            kc = jnp.concatenate([kc[8 * (b - b0):8 * (b - b0) + 8] for b in blocks], axis=0)
            sm = jnp.exp2(scores_mxu(kc, 2 * i + odd, odd, slice(qt * TQ, (qt + 1) * TQ), TQ))
            return {b: sm[16 * n:16 * n + 16] for n, b in enumerate(blocks)}

        def body(i, carry):
            T = 2 * NQ * NKC
            rows = chunk(i, FC)
            ps = {}
            extra = {}
            acc = bnd_acc
            for t in range(T + LAG):
                if t < T:
                    u, c = divmod(t, NKC)
                    odd, qt = divmod(u, NQ)
                    parts = p_vpu(odd, qt, c, extra)
                    blocks = list(range(KC // 16 - 1, len(parts) - 1, -1))
                    res = p_mxu(i, odd, qt, c, blocks[:SA])
                if t == T:
                    hh = ffn1(rows, 0, F1A)
                if t >= LAG:
                    ub, cb = divmod(t - LAG, NKC)
                    oddb, qtb = divmod(ub, NQ)
                    vt = vt_ref[2 * i + oddb, :, cb * KC:(cb + 1) * KC]
                    a = lax.dot_general(vt, ps.pop(t - LAG).astype(BF16), NN, preferred_element_type=F32)
                    acc = jnp.where(never_acc, acc, a) if cb == 0 else acc + a
                    if cb == NKC - 1:
                        store_o(acc, i, oddb, slice(qtb * TQ, (qtb + 1) * TQ))
                if t < T:
                    res.update(p_mxu(i, odd, qt, c, blocks[SA:]))
                    ps[t] = jnp.concatenate(parts + [res[b] for b in sorted(res)], axis=0)
            hh = jnp.concatenate([hh, ffn1(rows, F1A, FF)], axis=1)
            ffn2(rows, hh)
            pace = [hh[r:r + 8, c:c + LANES] for c in range(F1A, FF, LANES) for r in range(0, FC // 2, 8)]
            prep(jnp.minimum(i + 1, NP - 1), never, pace, NLH)
            return carry

        lax.fori_loop(0, NP, body, 0)

    @pl.when(jnp.logical_not(safe))
    def _fallback():
        def unit(u, carry):
            i = u // (S // TS)
            cols = chunk(u % (S // TS), TS)
            for odd in range(2):
                s = scores_mxu(k_ref[i], 2 * i + odd, odd, cols, TS)
                m = jnp.max(s, axis=0, keepdims=True)
                p = jnp.exp2(s - m).astype(BF16)
                acc = lax.dot_general(vt_ref[2 * i + odd], p, NN, preferred_element_type=F32)
                store_o(acc, i, odd, cols)
            return carry

        lax.fori_loop(0, NP * (S // TS), unit, 0)

        def ffn(i, carry):
            rows = chunk(i, 64)
            ffn2(rows, ffn1(rows, 0, FF))
            return carry

        lax.fori_loop(0, S // 64, ffn, 0)

    gw = gw_ref[...].astype(F32).reshape(1, -1)
    copies = []
    r0 = 0
    for n, sz in enumerate(OUT_CHUNKS):
        rows = pl.ds(r0, sz)
        r0 += sz
        o = ot_ref[:, rows].T.astype(BF16)
        a = jnp.dot(o, wo_ref[...], preferred_element_type=F32)
        z = jnp.sum(x_ref[rows, :].astype(F32) * gw, axis=-1, keepdims=True)
        g = 1.0 / (1.0 + jnp.exp(-z))
        o_ref[rows, :] = (g * a + (1.0 - g) * fb_ref[rows, :]).astype(o_ref.dtype)
        cp = pltpu.make_async_copy(o_ref.at[rows, :], o_hbm.at[0, rows, :], out_sem.at[n])
        cp.start()
        copies.append(cp)
    for cp in copies:
        cp.wait()


@jax.jit
def pallas_gated_mix__softmax_full_mha__dense_activation_squared_relu__prompt_kernel(
    A_x: jax.Array,
    A_wqkv: jax.Array,
    A_wo: jax.Array,
    B_x: jax.Array,
    B_w1: jax.Array,
    B_b1: jax.Array,
    B_w2: jax.Array,
    B_b2: jax.Array,
    gate_w: jax.Array,
):
    del B_x
    B, S, D = A_x.shape
    F = B_w1.shape[1]
    DH = D // H
    assert B == 1 and sum(OUT_CHUNKS) == S and DH == 20
    hbm = pl.BlockSpec(memory_space=pl.ANY)
    return pl.pallas_call(
        functools.partial(_kernel, S=S, D=D, DH=DH),
        out_shape=jax.ShapeDtypeStruct((B, S, D), A_x.dtype),
        in_specs=[hbm] * 8,
        out_specs=hbm,
        scratch_shapes=[
            pltpu.VMEM((S, D), BF16),
            pltpu.VMEM((3, D, D), BF16),
            pltpu.VMEM((D, D), BF16),
            pltpu.VMEM((D, F), BF16),
            pltpu.VMEM((F, D), BF16),
            pltpu.VMEM((S, D), BF16),
            pltpu.VMEM((D, S), F32),
            pltpu.VMEM((H // 2, S // 2, LANES), U32),
            pltpu.VMEM((H, 24, S), F32),
            pltpu.VMEM((D, S), F32),
            pltpu.VMEM((S, D), F32),
            pltpu.VMEM((2 * DH, (S // KC + XT) * VR, LANES), F32),
            pltpu.VMEM((2 * DH, 8, S), F32),
            pltpu.VMEM((H, 16, S), U32),
            pltpu.VMEM((8, D), F32),
            pltpu.VMEM((D, LANES), F32),
            pltpu.VMEM((F,), BF16),
            pltpu.VMEM((D,), BF16),
            pltpu.VMEM((D,), BF16),
            pltpu.SemaphoreType.DMA((9,)),
            pltpu.SemaphoreType.DMA((NK + 1,)),
            pltpu.SemaphoreType.DMA((len(OUT_CHUNKS),)),
        ],
        compiler_params=pltpu.CompilerParams(vmem_limit_bytes=100 * 1024 * 1024),
    )(A_x, A_wqkv, A_wo, B_w1, B_b1, B_w2, B_b2, gate_w)
```

```python
import functools
import math

import jax
import jax.numpy as jnp
from jax import lax
import jax.experimental.pallas as pl
import jax.experimental.pallas.tpu as pltpu

H = 32
LANES = 128
TQ = 512
KC = 128
VR = 16
XT = 2
LAG = 2
SA = 2
DC = 4
RC = 512
TS = 256
F1A = 512
NLH = 32
K0 = 320
NK = 2
OUT_CHUNKS = (512, 512, 512, 256, 128, 128)
SAFE_LOG2 = 40.0

NN = (((1,), (0,)), ((), ()))
F32 = jnp.float32
BF16 = jnp.bfloat16
U32 = jnp.uint32


def _kernel(x_hbm, wqkv_hbm, wo_hbm, w1_hbm, b1_hbm, w2_hbm, b2_hbm, gw_hbm,
            o_hbm,
            x_ref, wqkv_ref, wo_ref, w1_ref, w2_ref, o_ref,
            qt_ref, k_ref, vt_ref, ot_ref, fb_ref, kb_ref, qb_ref, qw_ref,
            mk_ref, mq_ref, b1_ref, b2_ref, gw_ref, in_sem, x_sem, out_sem, *, S, D, DH):
    NG = D // LANES
    NQ = S // TQ
    NKC = S // KC
    NR = S // RC
    NP = H // 2
    PW = 2 * DH
    FC = S // NP
    NJ = TQ // LANES
    FF = w1_ref.shape[1]
    KH = KC // 2
    qscale = (DH ** -0.5) * math.log2(math.e)
    xtiles = [(e + 1) * NKC // XT - 1 for e in range(XT)]
    assert 2 * NJ * XT == NKC

    def chunk(r, n=RC):
        return pl.ds(pl.multiple_of(r * n, n), n)

    def wcopy(n):
        return pltpu.make_async_copy(wqkv_hbm.at[:, pl.ds(n * D, D)], wqkv_ref.at[n], in_sem.at[n])

    KR = (S - K0) // NK
    assert KR * NK + K0 == S and KR % 16 == 0

    def krows(r, div=1):
        if isinstance(r, int) and r < 0:
            return pl.ds(0, K0 // div)
        return pl.ds(pl.multiple_of(K0 // div + r * (KR // div), 16 // div), KR // div)

    def xcopy(r):
        return pltpu.make_async_copy(x_hbm.at[0, krows(r), :], x_ref.at[krows(r), :], x_sem.at[r + 1])

    cp_wq, cp_wk, cp_wv = wcopy(0), wcopy(1), wcopy(2)
    cp_late = [pltpu.make_async_copy(a, b, in_sem.at[3 + n]) for n, (a, b) in enumerate((
        (w1_hbm, w1_ref), (w2_hbm, w2_ref), (wo_hbm, wo_ref),
        (b1_hbm, b1_ref), (b2_hbm, b2_ref), (gw_hbm, gw_ref)))]
    xcopy(-1).start()
    cp_wk.start()
    mk_ref[...] = jnp.zeros(mk_ref.shape, F32)
    mq_ref[...] = jnp.zeros(mq_ref.shape, F32)

    def prep(pair, never, pace, n_pace):
        src = jnp.concatenate(
            [k_ref[pair, c * KH:c * KH + VR // 2, :] for c in range(NKC)]
            + [k_ref[pair, c * KH + VR // 2:c * KH + VR, :] for c in xtiles], axis=0)
        kpace = []
        for d in range(PW):
            kb = jnp.broadcast_to(src[:, d:d + 1], src.shape)
            kb_ref[d] = pltpu.bitcast(kb, BF16).astype(F32)
            kpace.append(kb[0:8])
        base = pl.multiple_of(PW * pair, 8)
        nt = (PW // 8) * (S // LANES)
        n = 0
        for t in range(PW // 8):
            for j in range(S // LANES):
                win = qt_ref[pl.ds(base + 8 * t, 8), j * LANES:(j + 1) * LANES]
                if n < n_pace:
                    dep = pace[n * len(pace) // n_pace]
                else:
                    dep = kpace[(n - n_pace) * PW // (nt - n_pace)]
                win = jnp.where(never, pltpu.bitcast(dep, F32), win)
                n += 1
                qb_ref[8 * t:8 * t + 8, :, j * LANES:(j + 1) * LANES] = jnp.stack(
                    [jnp.broadcast_to(win[r:r + 1, :], (8, LANES)) for r in range(8)])

    def lane_fold_absmax(a):
        a = jnp.abs(a)
        out = a[:, 0:LANES]
        for j in range(1, a.shape[1] // LANES):
            out = jnp.maximum(out, a[:, j * LANES:(j + 1) * LANES])
        return out

    xcopy(-1).wait()
    xcopy(0).start()
    cp_wk.wait()
    for cp in [xcopy(r) for r in range(1, NK)] + [cp_wq, cp_wv]:
        cp.start()

    def proj_k(r, c, first=False):
        n = K0 if first else KR
        if not first:
            xcopy(r).wait()
        lane = lax.broadcasted_iota(jnp.int32, (n // 2, LANES), 1)
        mk = mk_ref[...]
        k = jnp.dot(x_ref[krows(r), :], wqkv_ref[1], preferred_element_type=F32)
        kp = pltpu.bitcast(k.astype(BF16), U32)
        grp = [kp[:, g * LANES:(g + 1) * LANES] for g in range(NG)]
        for p in range(NP):
            g, off = divmod(PW * p, LANES)
            t = grp[g]
            if off + PW > LANES:
                t = jnp.where(lane >= off, t, grp[g + 1])
            if off:
                t = pltpu.roll(t, LANES - off, 1)
            k_ref[p, krows(r, 2), :] = t
        mk_ref[...] = jnp.maximum(mk, jnp.max(jnp.abs(k).reshape(n // 8, 8, D), axis=0))
        return c

    proj_k(-1, 0, first=True)
    lax.fori_loop(0, NK, proj_k, 0)
    for cp in cp_late:
        cp.start()
    cp_wq.wait()
    cp_wv.wait()

    row24 = lax.broadcasted_iota(jnp.int32, (24, RC), 0)

    def proj_qv(r, mv, pace=None):
        rows = chunk(r)
        xc = x_ref[rows, :]
        qs, vs = [], []
        for j0 in range(0, D, LANES):
            q = jnp.dot(xc, wqkv_ref[0, :, j0:j0 + LANES], preferred_element_type=F32)
            qs.append((q * qscale).astype(BF16).astype(F32).T)
        for j0 in range(0, D, LANES):
            v = jnp.dot(xc, wqkv_ref[2, :, j0:j0 + LANES], preferred_element_type=F32)
            vs.append(v.astype(BF16).astype(F32).T)
            if pace is not None and j0 < D - LANES:
                pace += [v[r_:r_ + 8] for r_ in range(0, RC, 8)]
        qT = jnp.concatenate(qs, axis=0)
        vT = jnp.concatenate(vs, axis=0)
        qt_ref[:, rows] = qT
        zero8 = jnp.zeros((8, RC), F32)
        for h in range(H):
            odd = h % 2
            off = PW * (h // 2) + 16 * odd
            valid = (row24 >= 4) if odd else (row24 < DH)
            w = jnp.concatenate([jnp.where(valid, qT[off:off + 24, :], 0.0), zero8], axis=0)
            qw_ref[h, :, rows] = pltpu.bitcast(w.astype(BF16), U32)
            vt_ref[h, :, rows] = jnp.where(valid, vT[off:off + 24, :], 1.0)
        mq_ref[...] = jnp.maximum(mq_ref[...], lane_fold_absmax(qT))
        return jnp.maximum(mv, jnp.max(lane_fold_absmax(vT).reshape(D // 8, 8, LANES), axis=0))

    mv = lax.fori_loop(0, NR - 1, proj_qv, jnp.zeros((8, LANES), F32))
    for cp in cp_late:
        cp.wait()
    never0 = mv < 0.0
    pace0 = []
    mv = proj_qv(NR - 1, mv, pace0)
    prep(0, never0, pace0, (PW // 8) * (S // LANES))

    mk = jnp.max(mk_ref[...], axis=0, keepdims=True)
    col = lax.broadcasted_iota(jnp.int32, (H, D), 1)
    hrow = lax.broadcasted_iota(jnp.int32, (H, D), 0) * DH
    sel = jnp.where((col >= hrow) & (col < hrow + DH), mk, 0.0)
    bnd = jnp.dot(sel, mq_ref[...], preferred_element_type=F32)
    bnd = jnp.max(bnd.reshape(H // 8, 8, LANES), axis=0)
    vmax = jnp.max(mv)
    safe = (jnp.max(bnd) <= SAFE_LOG2) & (vmax <= 2.0 ** 60) & (vmax >= 2.0 ** -60)

    def ffn1(rows, c0, c1):
        b1 = b1_ref[...].astype(F32).reshape(1, -1)
        hh = jnp.dot(x_ref[rows, :], w1_ref[:, c0:c1], preferred_element_type=F32) + b1[:, c0:c1]
        hh = jnp.maximum(hh, 0.0)
        return pltpu.bitcast((hh * hh).astype(BF16), U32)

    def ffn2(rows, hh):
        b2 = b2_ref[...].astype(F32).reshape(1, -1)
        fb_ref[rows, :] = jnp.dot(pltpu.bitcast(hh, BF16), w2_ref[...], preferred_element_type=F32) + b2

    def scores_mxu(kc, h, odd, cols, width):
        w = qw_ref[h, :, cols]
        if odd:
            w = jnp.concatenate([jnp.zeros((8, width), U32), w], axis=0)
        w = pltpu.bitcast(w, BF16)
        return lax.dot_general(pltpu.bitcast(kc, BF16)[:, 0:w.shape[0]], w, NN, preferred_element_type=F32)

    def store_o(acc, pair, odd, cols):
        l = acc[0:1] if odd else acc[23:24]
        o = acc * (1.0 / l)
        base = pl.multiple_of(PW * pair, 8)
        if not odd:
            ot_ref[pl.ds(base, 24), cols] = o
        else:
            row8 = lax.broadcasted_iota(jnp.int32, (8, acc.shape[1]), 0)
            off = pl.multiple_of(base + 16, 8)
            old = ot_ref[pl.ds(off, 8), cols]
            ot_ref[pl.ds(off, 8), cols] = jnp.where(row8 >= 4, o[0:8], old)
            ot_ref[pl.ds(off + 8, 16), cols] = o[8:24]

    @pl.when(safe)
    def _fast():
        never = bnd < 0.0
        bnd_acc = jnp.tile(bnd, (3, NJ))
        never_acc = bnd_acc < 0.0

        def after(x, dep):
            return jnp.where(never[None], dep, x)

        def scores_vpu(kb, qb, start):
            acc = None
            for d in range(0, DH, DC):
                t = kb[d:d + DC] * qb[d:d + DC]
                if acc is not None:
                    t = jnp.concatenate([acc[None], t], axis=0)
                elif start is not None:
                    t = jnp.concatenate([after(t[0], start)[None], t[1:]], axis=0)
                acc = jnp.sum(t, axis=0)
            return acc

        def p_vpu(odd, qt, c, extra):
            dims = slice(odd * DH, (odd + 1) * DH)
            qb = qb_ref[dims, :, qt * TQ:(qt + 1) * TQ][:, None]
            kb = kb_ref[dims, c * VR:(c + 1) * VR, :].reshape(DH, VR // 8, 8, LANES)
            e, pos = divmod(c, 2 * NJ)
            jx, rx = divmod(pos, 2)
            rest = [j for j in range(NJ) if j != jx]
            cols = {}
            prev = None
            for j in rest[:2] + [jx] + rest[2:]:
                q = qb[..., j * LANES:(j + 1) * LANES]
                if j == jx:
                    r0 = (NKC + e) * VR + 8 * rx
                    kx = kb_ref[dims, r0:r0 + 8, :][:, None]
                    w = scores_vpu(jnp.concatenate([kb, kx], axis=1), q,
                                   jnp.concatenate([prev, prev[1:2]], axis=0))
                    extra[(j, rx)] = jnp.exp2(w[2])
                    cols[j] = w[0:2]
                    prev = jnp.concatenate([w[0:1], after(w[1:2], w[2:3])], axis=0)
                else:
                    prev = cols[j] = scores_vpu(kb, q, prev)
            parts = [jnp.exp2(jnp.concatenate([cols[j].reshape(VR, LANES) for j in range(NJ)], axis=1))]
            if c in xtiles:
                parts.append(jnp.concatenate(
                    [jnp.concatenate([extra.pop((j, r)) for j in range(NJ)], axis=1) for r in range(2)], axis=0))
            return parts

        def p_mxu(i, odd, qt, c, blocks):
            b0 = min(blocks)
            kc = k_ref[i, c * KH + 8 * b0:c * KH + 8 * (b0 + len(blocks)), :]
            kc = jnp.concatenate([kc[8 * (b - b0):8 * (b - b0) + 8] for b in blocks], axis=0)
            sm = jnp.exp2(scores_mxu(kc, 2 * i + odd, odd, slice(qt * TQ, (qt + 1) * TQ), TQ))
            return {b: sm[16 * n:16 * n + 16] for n, b in enumerate(blocks)}

        def body(i, carry):
            T = 2 * NQ * NKC
            rows = chunk(i, FC)
            ps = {}
            extra = {}
            acc = bnd_acc
            for t in range(T + LAG):
                if t < T:
                    u, c = divmod(t, NKC)
                    odd, qt = divmod(u, NQ)
                    parts = p_vpu(odd, qt, c, extra)
                    blocks = list(range(KC // 16 - 1, len(parts) - 1, -1))
                    res = p_mxu(i, odd, qt, c, blocks[:SA])
                if t == T:
                    hh = ffn1(rows, 0, F1A)
                if t >= LAG:
                    ub, cb = divmod(t - LAG, NKC)
                    oddb, qtb = divmod(ub, NQ)
                    vt = vt_ref[2 * i + oddb, :, cb * KC:(cb + 1) * KC]
                    a = lax.dot_general(vt, ps.pop(t - LAG).astype(BF16), NN, preferred_element_type=F32)
                    acc = jnp.where(never_acc, acc, a) if cb == 0 else acc + a
                    if cb == NKC - 1:
                        store_o(acc, i, oddb, slice(qtb * TQ, (qtb + 1) * TQ))
                if t < T:
                    res.update(p_mxu(i, odd, qt, c, blocks[SA:]))
                    ps[t] = jnp.concatenate(parts + [res[b] for b in sorted(res)], axis=0)
            hh = jnp.concatenate([hh, ffn1(rows, F1A, FF)], axis=1)
            ffn2(rows, hh)
            pace = [hh[r:r + 8, c:c + LANES] for c in range(F1A, FF, LANES) for r in range(0, FC // 2, 8)]
            prep(jnp.minimum(i + 1, NP - 1), never, pace, NLH)
            return carry

        lax.fori_loop(0, NP, body, 0)

    @pl.when(jnp.logical_not(safe))
    def _fallback():
        def unit(u, carry):
            i = u // (S // TS)
            cols = chunk(u % (S // TS), TS)
            for odd in range(2):
                s = scores_mxu(k_ref[i], 2 * i + odd, odd, cols, TS)
                m = jnp.max(s, axis=0, keepdims=True)
                p = jnp.exp2(s - m).astype(BF16)
                acc = lax.dot_general(vt_ref[2 * i + odd], p, NN, preferred_element_type=F32)
                store_o(acc, i, odd, cols)
            return carry

        lax.fori_loop(0, NP * (S // TS), unit, 0)

        def ffn(i, carry):
            rows = chunk(i, 64)
            ffn2(rows, ffn1(rows, 0, FF))
            return carry

        lax.fori_loop(0, S // 64, ffn, 0)

    gw = gw_ref[...].astype(F32).reshape(1, -1)
    copies = []
    r0 = 0
    for n, sz in enumerate(OUT_CHUNKS):
        rows = pl.ds(r0, sz)
        r0 += sz
        o = ot_ref[:, rows].T.astype(BF16)
        a = jnp.dot(o, wo_ref[...], preferred_element_type=F32)
        z = jnp.sum(x_ref[rows, :].astype(F32) * gw, axis=-1, keepdims=True)
        g = 1.0 / (1.0 + jnp.exp(-z))
        o_ref[rows, :] = (g * a + (1.0 - g) * fb_ref[rows, :]).astype(o_ref.dtype)
        cp = pltpu.make_async_copy(o_ref.at[rows, :], o_hbm.at[0, rows, :], out_sem.at[n])
        cp.start()
        copies.append(cp)
    for cp in copies:
        cp.wait()


@jax.jit
def pallas_gated_mix__softmax_full_mha__dense_activation_squared_relu__prompt_kernel(
    A_x: jax.Array,
    A_wqkv: jax.Array,
    A_wo: jax.Array,
    B_x: jax.Array,
    B_w1: jax.Array,
    B_b1: jax.Array,
    B_w2: jax.Array,
    B_b2: jax.Array,
    gate_w: jax.Array,
):
    del B_x
    B, S, D = A_x.shape
    F = B_w1.shape[1]
    DH = D // H
    assert B == 1 and sum(OUT_CHUNKS) == S and DH == 20
    hbm = pl.BlockSpec(memory_space=pl.ANY)
    return pl.pallas_call(
        functools.partial(_kernel, S=S, D=D, DH=DH),
        out_shape=jax.ShapeDtypeStruct((B, S, D), A_x.dtype),
        in_specs=[hbm] * 8,
        out_specs=hbm,
        scratch_shapes=[
            pltpu.VMEM((S, D), BF16),
            pltpu.VMEM((3, D, D), BF16),
            pltpu.VMEM((D, D), BF16),
            pltpu.VMEM((D, F), BF16),
            pltpu.VMEM((F, D), BF16),
            pltpu.VMEM((S, D), BF16),
            pltpu.VMEM((D, S), F32),
            pltpu.VMEM((H // 2, S // 2, LANES), U32),
            pltpu.VMEM((H, 24, S), F32),
            pltpu.VMEM((D, S), F32),
            pltpu.VMEM((S, D), F32),
            pltpu.VMEM((2 * DH, (S // KC + XT) * VR, LANES), F32),
            pltpu.VMEM((2 * DH, 8, S), F32),
            pltpu.VMEM((H, 16, S), U32),
            pltpu.VMEM((8, D), F32),
            pltpu.VMEM((D, LANES), F32),
            pltpu.VMEM((F,), BF16),
            pltpu.VMEM((D,), BF16),
            pltpu.VMEM((D,), BF16),
            pltpu.SemaphoreType.DMA((9,)),
            pltpu.SemaphoreType.DMA((NK + 1,)),
            pltpu.SemaphoreType.DMA((len(OUT_CHUNKS),)),
        ],
        compiler_params=pltpu.CompilerParams(vmem_limit_bytes=100 * 1024 * 1024),
    )(A_x, A_wqkv, A_wo, B_w1, B_b1, B_w2, B_b2, gate_w)
```

```python
import functools
import math

import jax
import jax.numpy as jnp
from jax import lax
import jax.experimental.pallas as pl
import jax.experimental.pallas.tpu as pltpu

H = 32
LANES = 128
TQ = 512
KC = 128
KB = 32
G = 12
LB = 7
RC = 512
TS = 256
F1A = 512
K0 = 320
NK = 2
OUT_CHUNKS = (512, 512, 512, 256, 128, 128)
SAFE_TERM = 3.0
TINY = 1e-30

NN = (((1,), (0,)), ((), ()))
F32 = jnp.float32
BF16 = jnp.bfloat16
U32 = jnp.uint32
I32 = jnp.int32
I8 = jnp.int8


def _rint(a):
    return jnp.round(a).astype(I32)


def _pack8(a):
    return pltpu.bitcast(a.astype(I8), U32)


def _kernel(x_hbm, wqkv_hbm, wo_hbm, w1_hbm, b1_hbm, w2_hbm, b2_hbm, gw_hbm,
            o_hbm,
            x_ref, wqkv_ref, wo_ref, w1_ref, w2_ref, o_ref,
            qt_ref, kf_ref, kl_ref, k8_ref, vt_ref, ot_ref, fb_ref, q8_ref, qs_ref,
            mk_ref, rk_ref, mkt_ref, b1_ref, b2_ref, gw_ref, in_sem, x_sem, out_sem, *, S, D, DH):
    NG = D // LANES
    NQ = S // TQ
    NKC = S // KC
    NR = S // RC
    NP = H // 2
    PW = 2 * DH
    FC = S // NP
    NJ = TQ // LANES
    FF = w1_ref.shape[1]
    KR = (S - K0) // NK
    assert KR * NK + K0 == S and KR % 16 == 0
    qscale = (DH ** -0.5) * math.log2(math.e)

    def chunk(r, n=RC):
        return pl.ds(pl.multiple_of(r * n, n), n)

    def krows(r):
        if r is None:
            return pl.ds(0, K0)
        return pl.ds(pl.multiple_of(K0 + r * KR, 16), KR)

    def xcopy(r):
        return pltpu.make_async_copy(x_hbm.at[0, krows(r), :], x_ref.at[krows(r), :],
                                     x_sem.at[NK if r is None else r])

    def wcopy(n):
        return pltpu.make_async_copy(wqkv_hbm.at[:, pl.ds(n * D, D)], wqkv_ref.at[n], in_sem.at[n])

    cp_wq, cp_wk, cp_wv = wcopy(0), wcopy(1), wcopy(2)
    cp_late = [pltpu.make_async_copy(a, b, in_sem.at[3 + n]) for n, (a, b) in enumerate((
        (w1_hbm, w1_ref), (w2_hbm, w2_ref), (wo_hbm, wo_ref),
        (b1_hbm, b1_ref), (b2_hbm, b2_ref), (gw_hbm, gw_ref)))]
    xcopy(None).start()
    cp_wk.start()
    mk_ref[...] = jnp.full(mk_ref.shape, TINY, F32)

    def group(h):
        lo = h * DH
        return lo, lo // LANES, (lo + DH - 1) // LANES

    def prep_k(pair):
        lane = lax.broadcasted_iota(I32, (S // 4, LANES), 1)
        is_a = (lane < 64) | ((lane >= 96) & (lane < 112))
        is_y = (lane < 80) | ((lane >= 112) & (lane < 116))
        for odd in range(2):
            lo, ga, gb = group(2 * pair + odd)
            g = jnp.where(ga == gb, ga, NG + ga)
            dim = jnp.where(lane < 96, (lane & 15) + 4 * odd, (lane & 3) + 16 * (1 - odd))
            idx = (lo + dim) & (LANES - 1)
            a, y, x = [jnp.take_along_axis(kl_ref[v, g], idx, axis=1, mode="promise_in_bounds")
                       for v in range(3)]
            k8_ref[odd] = jnp.where(is_a, a, jnp.where(is_y, y, x))

    def prep_q(pair, never, pace):
        row8 = lax.broadcasted_iota(I32, (8, LANES), 0)
        n = 0
        for odd in range(2):
            win = pl.ds(pl.multiple_of(PW * pair + 16 * odd, 8), 24)
            for j in range(S // LANES):
                cols = slice(j * LANES, (j + 1) * LANES)
                w = qt_ref[win, cols] * mkt_ref[win, :]
                if odd:
                    half, full = w[0:8], w[8:24]
                    half = jnp.where(row8 >= 4, half, pltpu.roll(half, 4, 0))
                else:
                    full, half = w[0:16], w[16:24]
                    half = jnp.where(row8 < 4, half, pltpu.roll(half, 4, 0))
                half = jnp.where(never, pace[n * len(pace) // (2 * S // LANES)], half)
                n += 1
                w = jnp.concatenate([full, half], axis=0)
                sq = jnp.maximum(jnp.max(jnp.abs(w), axis=0, keepdims=True), TINY)
                sq = jnp.broadcast_to(sq, (8, LANES))
                r = pl.reciprocal(sq, approx=True)
                r = r * (2.0 - sq * r) * 127.0
                t = w.reshape(3, 8, LANES) * r[None]
                a = _rint(t)
                af = a.astype(F32)
                xf = af * 0.125
                yf = (t - af) * 32.0
                x, y = _rint(xf[0:2]), _rint(yf[0:2])
                xy = _rint(jnp.where(row8 < 4, xf[2], yf[2]))
                q8_ref[odd, :, cols] = _pack8(jnp.concatenate(
                    [a[0], a[1], a[0], a[1], x[0], x[1], y[0], y[1],
                     a[2], a[2], xy, jnp.zeros((8, LANES), I32)], axis=0))
                qs_ref[odd, :, cols] = sq * (1.0 / (4.0 * 127.0 * 127.0))

    xcopy(None).wait()
    xcopy(0).start()
    cp_wk.wait()
    for cp in [xcopy(r) for r in range(1, NK)] + [cp_wq, cp_wv]:
        cp.start()

    def proj_k(r, c):
        if r is not None:
            xcopy(r).wait()
        mk = mk_ref[...]
        k = jnp.dot(x_ref[krows(r), :], wqkv_ref[1], preferred_element_type=F32)
        kf_ref[krows(r), :] = k
        mk_ref[...] = jnp.maximum(mk, jnp.max(jnp.abs(k).reshape(k.shape[0] // 8, 8, D), axis=0))
        return c

    proj_k(None, 0)
    lax.fori_loop(0, NK, proj_k, 0)
    for cp in cp_late:
        cp.start()
    mk = jnp.max(mk_ref[...], axis=0, keepdims=True)
    mk_ref[...] = jnp.broadcast_to(mk, (8, D))
    rk_ref[...] = jnp.broadcast_to(127.0 / mk, (8, D))
    cp_wq.wait()
    cp_wv.wait()

    row24 = lax.broadcasted_iota(I32, (24, RC), 0)

    def proj_qv(r, carry, out=None):
        term, mv = carry
        never = term < 0.0
        rows = chunk(r)
        xc = x_ref[rows, :]
        qs, vs, pace = [], [], []
        for j0 in range(0, D, LANES):
            q = jnp.dot(xc, wqkv_ref[0, :, j0:j0 + LANES], preferred_element_type=F32)
            pace += [q[r_:r_ + 8] for r_ in range(0, RC, 8)]
            q = q * qscale
            mq = jnp.max(jnp.abs(q).reshape(RC // 8, 8, LANES), axis=0)
            term = jnp.maximum(term, mq * mk_ref[:, j0:j0 + LANES])
            qs.append(q.T)
        for j0 in range(0, D, LANES):
            v = jnp.dot(xc, wqkv_ref[2, :, j0:j0 + LANES], preferred_element_type=F32)
            pace += [v[r_:r_ + 8] for r_ in range(0, RC, 8)]
            mv = jnp.maximum(mv, jnp.max(jnp.abs(v).reshape(RC // 8, 8, LANES), axis=0))
            vs.append(v.astype(BF16).astype(F32).T)
        qt_ref[:, rows] = jnp.concatenate(qs, axis=0)
        vT = jnp.concatenate(vs, axis=0)
        for h in range(H):
            odd = h % 2
            off = PW * (h // 2) + 16 * odd
            valid = (row24 >= 4) if odd else (row24 < DH)
            vt_ref[h, :, rows] = jnp.where(valid, vT[off:off + 24, :], 1.0)
        n_pace = len(pace) * (9 if out is None else 5) // 10
        lane = lax.broadcasted_iota(I32, (8, LANES), 1)
        n = 0
        for b in range(RC // KB):
            r0 = pl.multiple_of(r * RC + KB * b, KB)
            limbs = [[], [], []]
            for g in range(NG):
                cols = slice(g * LANES, (g + 1) * LANES)
                rk = jnp.where(never, pace[n * n_pace // (NG * RC // KB)], rk_ref[:, cols])
                n += 1
                t = (kf_ref[pl.ds(r0, KB), cols].reshape(4, 8, LANES) * rk[None]).reshape(KB, LANES)
                a = _rint(t)
                limbs[0].append(_pack8(a))
                limbs[1].append(_pack8(_rint((t - a.astype(F32)) * 32.0)))
                limbs[2].append(_pack8(_rint(t * 0.125)))
            for v, grp in enumerate(limbs):
                grp = grp + [jnp.where(lane >= LANES // 2, grp[g], grp[g + 1]) for g in range(NG - 1)]
                kl_ref[v, :, pl.ds(pl.multiple_of(r * (RC // 4) + 8 * b, 8), 8), :] = jnp.stack(grp)
        if out is not None:
            out += pace[6 * len(pace) // 10:9 * len(pace) // 10]
        return term, mv

    zero8 = jnp.zeros((8, LANES), F32)
    carry = lax.fori_loop(0, NR - 1, proj_qv, (zero8, zero8))
    for cp in cp_late:
        cp.wait()
    mkt_ref[...] = jnp.broadcast_to(mk_ref[0:1, :], (LANES, D)).T
    pace0 = []
    term, mv = proj_qv(NR - 1, carry, pace0)
    prep_k(0)
    prep_q(0, carry[0] < 0.0, pace0)
    vmax = jnp.max(mv)
    safe = (jnp.max(term) <= SAFE_TERM) & (vmax <= 2.0 ** 40) & (vmax >= 2.0 ** -40)

    def ffn1(rows, c0, c1):
        b1 = b1_ref[...].astype(F32).reshape(1, -1)
        hh = jnp.dot(x_ref[rows, :], w1_ref[:, c0:c1], preferred_element_type=F32) + b1[:, c0:c1]
        hh = jnp.maximum(hh, 0.0)
        return hh * hh

    def ffn2(rows, hh):
        b2 = b2_ref[...].astype(F32).reshape(1, -1)
        fb_ref[rows, :] = jnp.dot(hh.astype(BF16), w2_ref[...], preferred_element_type=F32) + b2

    def store_o(acc, pair, odd, cols):
        l = acc[0:1] if odd else acc[23:24]
        o = acc * (1.0 / l)
        base = pl.multiple_of(PW * pair, 8)
        if not odd:
            ot_ref[pl.ds(base, 24), cols] = o
        else:
            row8 = lax.broadcasted_iota(I32, (8, acc.shape[1]), 0)
            off = pl.multiple_of(base + 16, 8)
            old = ot_ref[pl.ds(off, 8), cols]
            ot_ref[pl.ds(off, 8), cols] = jnp.where(row8 >= 4, o[0:8], old)
            ot_ref[pl.ds(off + 8, 16), cols] = o[8:24]

    @pl.when(safe)
    def _fast():
        never = term < 0.0
        acc0 = jnp.tile(term, (3, NJ))
        never_acc = acc0 < 0.0
        BT = KC // KB

        def p_blocks(u, pos):
            odd, qt = divmod(u, NQ)
            cols = slice(qt * TQ, (qt + 1) * TQ)
            blocks = [BT * (b // BT) + BT - 1 - b % BT for b in pos]
            b0 = min(blocks)
            kc = k8_ref[odd, 8 * b0:8 * (max(blocks) + 1), :]
            kc = jnp.concatenate([kc[8 * (b - b0):8 * (b - b0) + 8] for b in blocks], axis=0)
            w = q8_ref[odd, :, cols]
            w = jnp.concatenate([w[0:8], w], axis=0)
            s = lax.dot_general(pltpu.bitcast(kc, I8), pltpu.bitcast(w, I8), NN, preferred_element_type=I32)
            s = s.astype(F32).reshape(4 * len(pos), 8, TQ) * qs_ref[odd, :, cols][None]
            p = jnp.exp2(s).reshape(KB * len(pos), TQ)
            return {(u, b): p[KB * n:KB * (n + 1)] for n, b in enumerate(blocks)}

        def body(i, carry):
            NB = BT * NKC
            TB = 2 * NQ * NB
            rows = chunk(i, FC)
            ps = {}
            acc = acc0
            done = 0
            t = 0
            while done < TB // BT:
                if t < TB:
                    t1 = min(TB, t + (G + LB % BT if t == 0 else G))
                    while t < t1:
                        u, b = divmod(t, NB)
                        n = min(t1 - t, NB - b)
                        ps.update(p_blocks(u, list(range(b, b + n))))
                        t += n
                else:
                    hh = ffn1(rows, 0, F1A)
                    t += LB
                while BT * (done + 1) + LB <= t:
                    u, c = divmod(done, NKC)
                    odd, qt = divmod(u, NQ)
                    vt = vt_ref[2 * i + odd, :, c * KC:(c + 1) * KC]
                    p = jnp.concatenate([ps.pop((u, BT * c + n)) for n in range(BT)], axis=0)
                    a = lax.dot_general(vt, p.astype(BF16), NN, preferred_element_type=F32)
                    acc = jnp.where(never_acc, acc, a) if c == 0 else acc + a
                    if c == NKC - 1:
                        store_o(acc, i, odd, slice(qt * TQ, (qt + 1) * TQ))
                    done += 1
            hh = jnp.concatenate([hh, ffn1(rows, F1A, FF)], axis=1)
            ffn2(rows, hh)
            nxt = jnp.minimum(i + 1, NP - 1)
            prep_k(nxt)
            prep_q(nxt, never, [hh[r:r + 8, c:c + LANES] for c in range(F1A, FF, LANES) for r in range(0, FC, 8)])
            return carry

        lax.fori_loop(0, NP, body, 0)

    @pl.when(jnp.logical_not(safe))
    def _fallback():
        lane = lax.broadcasted_iota(I32, (S, LANES), 1)
        rowi = lax.broadcasted_iota(I32, (LANES, TS), 0)

        def unit(u, carry):
            i = u // (S // TS)
            cols = chunk(u % (S // TS), TS)
            for odd in range(2):
                lo, ga, gb = group(2 * i + odd)
                off = lo & (LANES - 1)
                ca, cb = chunk(ga, LANES), chunk(gb, LANES)
                k = jnp.where(lane >= off, kf_ref[:, ca], kf_ref[:, cb])
                w = jnp.where(rowi >= off, qt_ref[ca, cols], qt_ref[cb, cols])
                w = jnp.where(((rowi - lo) & (LANES - 1)) < DH, w, 0.0)
                s = jnp.dot(k.astype(BF16), w.astype(BF16), preferred_element_type=F32)
                m = jnp.max(s, axis=0, keepdims=True)
                p = jnp.exp2(s - m).astype(BF16)
                acc = lax.dot_general(vt_ref[2 * i + odd], p, NN, preferred_element_type=F32)
                store_o(acc, i, odd, cols)
            return carry

        lax.fori_loop(0, NP * (S // TS), unit, 0)

        def ffn(i, carry):
            rows = chunk(i, 64)
            ffn2(rows, ffn1(rows, 0, FF))
            return carry

        lax.fori_loop(0, S // 64, ffn, 0)

    gw = gw_ref[...].astype(F32).reshape(1, -1)
    copies = []
    r0 = 0
    for n, sz in enumerate(OUT_CHUNKS):
        rows = pl.ds(r0, sz)
        r0 += sz
        o = ot_ref[:, rows].T.astype(BF16)
        a = jnp.dot(o, wo_ref[...], preferred_element_type=F32)
        z = jnp.sum(x_ref[rows, :].astype(F32) * gw, axis=-1, keepdims=True)
        g = 1.0 / (1.0 + jnp.exp(-z))
        o_ref[rows, :] = (g * a + (1.0 - g) * fb_ref[rows, :]).astype(o_ref.dtype)
        cp = pltpu.make_async_copy(o_ref.at[rows, :], o_hbm.at[0, rows, :], out_sem.at[n])
        cp.start()
        copies.append(cp)
    for cp in copies:
        cp.wait()


@jax.jit
def pallas_gated_mix__softmax_full_mha__dense_activation_squared_relu__prompt_kernel(
    A_x: jax.Array,
    A_wqkv: jax.Array,
    A_wo: jax.Array,
    B_x: jax.Array,
    B_w1: jax.Array,
    B_b1: jax.Array,
    B_w2: jax.Array,
    B_b2: jax.Array,
    gate_w: jax.Array,
):
    del B_x
    B, S, D = A_x.shape
    F = B_w1.shape[1]
    DH = D // H
    NG = D // LANES
    assert B == 1 and sum(OUT_CHUNKS) == S and DH == 20
    hbm = pl.BlockSpec(memory_space=pl.ANY)
    return pl.pallas_call(
        functools.partial(_kernel, S=S, D=D, DH=DH),
        out_shape=jax.ShapeDtypeStruct((B, S, D), A_x.dtype),
        in_specs=[hbm] * 8,
        out_specs=hbm,
        scratch_shapes=[
            pltpu.VMEM((S, D), BF16),
            pltpu.VMEM((3, D, D), BF16),
            pltpu.VMEM((D, D), BF16),
            pltpu.VMEM((D, F), BF16),
            pltpu.VMEM((F, D), BF16),
            pltpu.VMEM((S, D), BF16),
            pltpu.VMEM((D, S), F32),
            pltpu.VMEM((S, D), F32),
            pltpu.VMEM((3, 2 * NG - 1, S // 4, LANES), U32),
            pltpu.VMEM((2, S // 4, LANES), U32),
            pltpu.VMEM((H, 24, S), F32),
            pltpu.VMEM((D, S), F32),
            pltpu.VMEM((S, D), F32),
            pltpu.VMEM((2, 24, S), U32),
            pltpu.VMEM((2, 8, S), F32),
            pltpu.VMEM((8, D), F32),
            pltpu.VMEM((8, D), F32),
            pltpu.VMEM((D, LANES), F32),
            pltpu.VMEM((F,), BF16),
            pltpu.VMEM((D,), BF16),
            pltpu.VMEM((D,), BF16),
            pltpu.SemaphoreType.DMA((9,)),
            pltpu.SemaphoreType.DMA((NK + 1,)),
            pltpu.SemaphoreType.DMA((len(OUT_CHUNKS),)),
        ],
        compiler_params=pltpu.CompilerParams(vmem_limit_bytes=100 * 1024 * 1024),
    )(A_x, A_wqkv, A_wo, B_w1, B_b1, B_w2, B_b2, gate_w)
```

```python
import functools
import math

import jax
import jax.numpy as jnp
from jax import lax
import jax.experimental.pallas as pl
import jax.experimental.pallas.tpu as pltpu

H = 32
LANES = 128
TQ = 512
KC = 128
KB = 32
G = 12
LB = 7
RC = 512
TS = 256
F1A = 512
K0 = 320
NK = 2
OUT_CHUNKS = (512, 512, 512, 256, 128, 128)
SAFE_TERM = 3.0
TINY = 1e-30

NN = (((1,), (0,)), ((), ()))
F32 = jnp.float32
BF16 = jnp.bfloat16
U32 = jnp.uint32
I32 = jnp.int32
I8 = jnp.int8


def _rint(a):
    return jnp.round(a).astype(I32)


def _pack8(a):
    return pltpu.bitcast(a.astype(I8), U32)


def _kernel(x_hbm, wqkv_hbm, wo_hbm, w1_hbm, b1_hbm, w2_hbm, b2_hbm, gw_hbm,
            o_hbm,
            x_ref, wqkv_ref, wo_ref, w1_ref, w2_ref, o_ref,
            qt_ref, kf_ref, kl_ref, k8_ref, vt_ref, ot_ref, fb_ref, q8_ref, qs_ref,
            mk_ref, rk_ref, mkt_ref, b1_ref, b2_ref, gw_ref, in_sem, x_sem, out_sem, *, S, D, DH):
    NG = D // LANES
    NQ = S // TQ
    NKC = S // KC
    NR = S // RC
    NP = H // 2
    PW = 2 * DH
    FC = S // NP
    NJ = TQ // LANES
    FF = w1_ref.shape[1]
    KR = (S - K0) // NK
    assert KR * NK + K0 == S and KR % 16 == 0
    qscale = (DH ** -0.5) * math.log2(math.e)

    def chunk(r, n=RC):
        return pl.ds(pl.multiple_of(r * n, n), n)

    def krows(r):
        if r is None:
            return pl.ds(0, K0)
        return pl.ds(pl.multiple_of(K0 + r * KR, 16), KR)

    def xcopy(r):
        return pltpu.make_async_copy(x_hbm.at[0, krows(r), :], x_ref.at[krows(r), :],
                                     x_sem.at[NK if r is None else r])

    def wcopy(n):
        return pltpu.make_async_copy(wqkv_hbm.at[:, pl.ds(n * D, D)], wqkv_ref.at[n], in_sem.at[n])

    cp_wq, cp_wk, cp_wv = wcopy(0), wcopy(1), wcopy(2)
    cp_late = [pltpu.make_async_copy(a, b, in_sem.at[3 + n]) for n, (a, b) in enumerate((
        (w1_hbm, w1_ref), (w2_hbm, w2_ref), (wo_hbm, wo_ref),
        (b1_hbm, b1_ref), (b2_hbm, b2_ref), (gw_hbm, gw_ref)))]
    xcopy(None).start()
    cp_wk.start()
    mk_ref[...] = jnp.full(mk_ref.shape, TINY, F32)

    def group(h):
        lo = h * DH
        return lo, lo // LANES, (lo + DH - 1) // LANES

    def prep_k(pair):
        lane = lax.broadcasted_iota(I32, (S // 4, LANES), 1)
        is_a = (lane < 64) | ((lane >= 96) & (lane < 112))
        is_y = (lane < 80) | ((lane >= 112) & (lane < 116))
        for odd in range(2):
            lo, ga, gb = group(2 * pair + odd)
            g = jnp.where(ga == gb, ga, NG + ga)
            dim = jnp.where(lane < 96, (lane & 15) + 4 * odd, (lane & 3) + 16 * (1 - odd))
            idx = (lo + dim) & (LANES - 1)
            a, y, x = [jnp.take_along_axis(kl_ref[v, g], idx, axis=1, mode="promise_in_bounds")
                       for v in range(3)]
            k8_ref[odd] = jnp.where(is_a, a, jnp.where(is_y, y, x))

    def prep_q(pair, never, pace):
        row8 = lax.broadcasted_iota(I32, (8, LANES), 0)
        n = 0
        for odd in range(2):
            win = pl.ds(pl.multiple_of(PW * pair + 16 * odd, 8), 24)
            for j in range(S // LANES):
                cols = slice(j * LANES, (j + 1) * LANES)
                w = qt_ref[win, cols] * mkt_ref[win, :]
                if odd:
                    half, full = w[0:8], w[8:24]
                    half = jnp.where(row8 >= 4, half, pltpu.roll(half, 4, 0))
                else:
                    full, half = w[0:16], w[16:24]
                    half = jnp.where(row8 < 4, half, pltpu.roll(half, 4, 0))
                half = jnp.where(never, pace[n * len(pace) // (2 * S // LANES)], half)
                n += 1
                w = jnp.concatenate([full, half], axis=0)
                sq = jnp.maximum(jnp.max(jnp.abs(w), axis=0, keepdims=True), TINY)
                sq = jnp.broadcast_to(sq, (8, LANES))
                t = w.reshape(3, 8, LANES) * (127.0 / sq)[None]
                a = _rint(t)
                af = a.astype(F32)
                xf = af * 0.125
                yf = (t - af) * 32.0
                x, y = _rint(xf[0:2]), _rint(yf[0:2])
                xy = _rint(jnp.where(row8 < 4, xf[2], yf[2]))
                q8_ref[odd, :, cols] = _pack8(jnp.concatenate(
                    [a[0], a[1], a[0], a[1], x[0], x[1], y[0], y[1],
                     a[2], a[2], xy, jnp.zeros((8, LANES), I32)], axis=0))
                qs_ref[odd, :, cols] = sq * (1.0 / (4.0 * 127.0 * 127.0))

    xcopy(None).wait()
    xcopy(0).start()
    cp_wk.wait()
    for cp in [xcopy(r) for r in range(1, NK)] + [cp_wq, cp_wv]:
        cp.start()

    def proj_k(r, c):
        if r is not None:
            xcopy(r).wait()
        mk = mk_ref[...]
        k = jnp.dot(x_ref[krows(r), :], wqkv_ref[1], preferred_element_type=F32)
        kf_ref[krows(r), :] = k
        mk_ref[...] = jnp.maximum(mk, jnp.max(jnp.abs(k).reshape(k.shape[0] // 8, 8, D), axis=0))
        return c

    proj_k(None, 0)
    lax.fori_loop(0, NK, proj_k, 0)
    for cp in cp_late:
        cp.start()
    mk = jnp.max(mk_ref[...], axis=0, keepdims=True)
    mk_ref[...] = jnp.broadcast_to(mk, (8, D))
    rk_ref[...] = jnp.broadcast_to(127.0 / mk, (8, D))
    cp_wq.wait()
    cp_wv.wait()

    row24 = lax.broadcasted_iota(I32, (24, RC), 0)

    def proj_qv(r, carry, out=None):
        term, mv = carry
        never = term < 0.0
        rows = chunk(r)
        xc = x_ref[rows, :]
        qs, vs, pace = [], [], []
        if out is None:
            mkt_ref[...] = jnp.broadcast_to(mk_ref[0:1, :], (LANES, D)).T
        for j0 in range(0, D, LANES):
            q = jnp.dot(xc, wqkv_ref[0, :, j0:j0 + LANES], preferred_element_type=F32)
            pace += [q[r_:r_ + 8] for r_ in range(0, RC, 8)]
            q = q * qscale
            mq = jnp.max(jnp.abs(q).reshape(RC // 8, 8, LANES), axis=0)
            term = jnp.maximum(term, mq * mk_ref[:, j0:j0 + LANES])
            qs.append(q.T)
        for j0 in range(0, D, LANES):
            v = jnp.dot(xc, wqkv_ref[2, :, j0:j0 + LANES], preferred_element_type=F32)
            pace += [v[r_:r_ + 8] for r_ in range(0, RC, 8)]
            mv = jnp.maximum(mv, jnp.max(jnp.abs(v).reshape(RC // 8, 8, LANES), axis=0))
            vs.append(v.astype(BF16).astype(F32).T)
        qt_ref[:, rows] = jnp.concatenate(qs, axis=0)
        vT = jnp.concatenate(vs, axis=0)
        for h in range(H):
            odd = h % 2
            off = PW * (h // 2) + 16 * odd
            valid = (row24 >= 4) if odd else (row24 < DH)
            vt_ref[h, :, rows] = jnp.where(valid, vT[off:off + 24, :], 1.0)
        n_pace = len(pace) * (9 if out is None else 5) // 10
        lane = lax.broadcasted_iota(I32, (8, LANES), 1)
        n = 0
        for b in range(RC // KB):
            r0 = pl.multiple_of(r * RC + KB * b, KB)
            limbs = [[], [], []]
            for g in range(NG):
                cols = slice(g * LANES, (g + 1) * LANES)
                rk = jnp.where(never, pace[n * n_pace // (NG * RC // KB)], rk_ref[:, cols])
                n += 1
                t = (kf_ref[pl.ds(r0, KB), cols].reshape(4, 8, LANES) * rk[None]).reshape(KB, LANES)
                a = _rint(t)
                limbs[0].append(_pack8(a))
                limbs[1].append(_pack8(_rint((t - a.astype(F32)) * 32.0)))
                limbs[2].append(_pack8(_rint(t * 0.125)))
            for v, grp in enumerate(limbs):
                grp = grp + [jnp.where(lane >= LANES // 2, grp[g], grp[g + 1]) for g in range(NG - 1)]
                kl_ref[v, :, pl.ds(pl.multiple_of(r * (RC // 4) + 8 * b, 8), 8), :] = jnp.stack(grp)
        if out is not None:
            out += pace[6 * len(pace) // 10:9 * len(pace) // 10]
        return term, mv

    zero8 = jnp.zeros((8, LANES), F32)
    carry = lax.fori_loop(0, NR - 1, proj_qv, (zero8, zero8))
    for cp in cp_late:
        cp.wait()
    pace0 = []
    term, mv = proj_qv(NR - 1, carry, pace0)
    prep_k(0)
    prep_q(0, carry[0] < 0.0, pace0)
    vmax = jnp.max(mv)
    safe = (jnp.max(term) <= SAFE_TERM) & (vmax <= 2.0 ** 40) & (vmax >= 2.0 ** -40)

    def ffn1(rows, c0, c1):
        b1 = b1_ref[...].astype(F32).reshape(1, -1)
        hh = jnp.dot(x_ref[rows, :], w1_ref[:, c0:c1], preferred_element_type=F32) + b1[:, c0:c1]
        hh = jnp.maximum(hh, 0.0)
        return hh * hh

    def ffn2(rows, hh):
        b2 = b2_ref[...].astype(F32).reshape(1, -1)
        fb_ref[rows, :] = jnp.dot(hh.astype(BF16), w2_ref[...], preferred_element_type=F32) + b2

    def store_o(acc, pair, odd, cols):
        l = acc[0:1] if odd else acc[23:24]
        o = acc * (1.0 / l)
        base = pl.multiple_of(PW * pair, 8)
        if not odd:
            ot_ref[pl.ds(base, 24), cols] = o
        else:
            row8 = lax.broadcasted_iota(I32, (8, acc.shape[1]), 0)
            off = pl.multiple_of(base + 16, 8)
            old = ot_ref[pl.ds(off, 8), cols]
            ot_ref[pl.ds(off, 8), cols] = jnp.where(row8 >= 4, o[0:8], old)
            ot_ref[pl.ds(off + 8, 16), cols] = o[8:24]

    @pl.when(safe)
    def _fast():
        never = term < 0.0
        acc0 = jnp.tile(term, (3, NJ))
        never_acc = acc0 < 0.0
        BT = KC // KB

        def p_blocks(u, pos):
            odd, qt = divmod(u, NQ)
            cols = slice(qt * TQ, (qt + 1) * TQ)
            blocks = [BT * (b // BT) + BT - 1 - b % BT for b in pos]
            b0 = min(blocks)
            kc = k8_ref[odd, 8 * b0:8 * (max(blocks) + 1), :]
            kc = jnp.concatenate([kc[8 * (b - b0):8 * (b - b0) + 8] for b in blocks], axis=0)
            w = q8_ref[odd, :, cols]
            w = jnp.concatenate([w[0:8], w], axis=0)
            s = lax.dot_general(pltpu.bitcast(kc, I8), pltpu.bitcast(w, I8), NN, preferred_element_type=I32)
            s = s.astype(F32).reshape(4 * len(pos), 8, TQ) * qs_ref[odd, :, cols][None]
            p = jnp.exp2(s).reshape(KB * len(pos), TQ)
            return {(u, b): p[KB * n:KB * (n + 1)] for n, b in enumerate(blocks)}

        def body(i, carry):
            NB = BT * NKC
            TB = 2 * NQ * NB
            rows = chunk(i, FC)
            ps = {}
            acc = acc0
            done = 0
            t = 0
            while done < TB // BT:
                if t < TB:
                    t1 = min(TB, t + (G + LB % BT if t == 0 else G))
                    while t < t1:
                        u, b = divmod(t, NB)
                        n = min(t1 - t, NB - b)
                        ps.update(p_blocks(u, list(range(b, b + n))))
                        t += n
                else:
                    hh = ffn1(rows, 0, F1A)
                    t += LB
                while BT * (done + 1) + LB <= t:
                    u, c = divmod(done, NKC)
                    odd, qt = divmod(u, NQ)
                    vt = vt_ref[2 * i + odd, :, c * KC:(c + 1) * KC]
                    p = jnp.concatenate([ps.pop((u, BT * c + n)) for n in range(BT)], axis=0)
                    a = lax.dot_general(vt, p.astype(BF16), NN, preferred_element_type=F32)
                    acc = jnp.where(never_acc, acc, a) if c == 0 else acc + a
                    if c == NKC - 1:
                        store_o(acc, i, odd, slice(qt * TQ, (qt + 1) * TQ))
                    done += 1
            hh = jnp.concatenate([hh, ffn1(rows, F1A, FF)], axis=1)
            ffn2(rows, hh)
            nxt = jnp.minimum(i + 1, NP - 1)
            prep_k(nxt)
            prep_q(nxt, never, [hh[r:r + 8, c:c + LANES] for c in range(F1A, FF, LANES) for r in range(0, FC, 8)])
            return carry

        lax.fori_loop(0, NP, body, 0)

    @pl.when(jnp.logical_not(safe))
    def _fallback():
        lane = lax.broadcasted_iota(I32, (S, LANES), 1)
        rowi = lax.broadcasted_iota(I32, (LANES, TS), 0)

        def unit(u, carry):
            i = u // (S // TS)
            cols = chunk(u % (S // TS), TS)
            for odd in range(2):
                lo, ga, gb = group(2 * i + odd)
                off = lo & (LANES - 1)
                ca, cb = chunk(ga, LANES), chunk(gb, LANES)
                k = jnp.where(lane >= off, kf_ref[:, ca], kf_ref[:, cb])
                w = jnp.where(rowi >= off, qt_ref[ca, cols], qt_ref[cb, cols])
                w = jnp.where(((rowi - lo) & (LANES - 1)) < DH, w, 0.0)
                s = jnp.dot(k.astype(BF16), w.astype(BF16), preferred_element_type=F32)
                m = jnp.max(s, axis=0, keepdims=True)
                p = jnp.exp2(s - m).astype(BF16)
                acc = lax.dot_general(vt_ref[2 * i + odd], p, NN, preferred_element_type=F32)
                store_o(acc, i, odd, cols)
            return carry

        lax.fori_loop(0, NP * (S // TS), unit, 0)

        def ffn(i, carry):
            rows = chunk(i, 64)
            ffn2(rows, ffn1(rows, 0, FF))
            return carry

        lax.fori_loop(0, S // 64, ffn, 0)

    gw = gw_ref[...].astype(F32).reshape(1, -1)
    copies = []
    r0 = 0
    for n, sz in enumerate(OUT_CHUNKS):
        rows = pl.ds(r0, sz)
        r0 += sz
        o = ot_ref[:, rows].T.astype(BF16)
        a = jnp.dot(o, wo_ref[...], preferred_element_type=F32)
        z = jnp.sum(x_ref[rows, :].astype(F32) * gw, axis=-1, keepdims=True)
        g = 1.0 / (1.0 + jnp.exp(-z))
        o_ref[rows, :] = (g * a + (1.0 - g) * fb_ref[rows, :]).astype(o_ref.dtype)
        cp = pltpu.make_async_copy(o_ref.at[rows, :], o_hbm.at[0, rows, :], out_sem.at[n])
        cp.start()
        copies.append(cp)
    for cp in copies:
        cp.wait()


@jax.jit
def pallas_gated_mix__softmax_full_mha__dense_activation_squared_relu__prompt_kernel(
    A_x: jax.Array,
    A_wqkv: jax.Array,
    A_wo: jax.Array,
    B_x: jax.Array,
    B_w1: jax.Array,
    B_b1: jax.Array,
    B_w2: jax.Array,
    B_b2: jax.Array,
    gate_w: jax.Array,
):
    del B_x
    B, S, D = A_x.shape
    F = B_w1.shape[1]
    DH = D // H
    NG = D // LANES
    assert B == 1 and sum(OUT_CHUNKS) == S and DH == 20
    hbm = pl.BlockSpec(memory_space=pl.ANY)
    return pl.pallas_call(
        functools.partial(_kernel, S=S, D=D, DH=DH),
        out_shape=jax.ShapeDtypeStruct((B, S, D), A_x.dtype),
        in_specs=[hbm] * 8,
        out_specs=hbm,
        scratch_shapes=[
            pltpu.VMEM((S, D), BF16),
            pltpu.VMEM((3, D, D), BF16),
            pltpu.VMEM((D, D), BF16),
            pltpu.VMEM((D, F), BF16),
            pltpu.VMEM((F, D), BF16),
            pltpu.VMEM((S, D), BF16),
            pltpu.VMEM((D, S), F32),
            pltpu.VMEM((S, D), F32),
            pltpu.VMEM((3, 2 * NG - 1, S // 4, LANES), U32),
            pltpu.VMEM((2, S // 4, LANES), U32),
            pltpu.VMEM((H, 24, S), F32),
            pltpu.VMEM((D, S), F32),
            pltpu.VMEM((S, D), F32),
            pltpu.VMEM((2, 24, S), U32),
            pltpu.VMEM((2, 8, S), F32),
            pltpu.VMEM((8, D), F32),
            pltpu.VMEM((8, D), F32),
            pltpu.VMEM((D, LANES), F32),
            pltpu.VMEM((F,), BF16),
            pltpu.VMEM((D,), BF16),
            pltpu.VMEM((D,), BF16),
            pltpu.SemaphoreType.DMA((9,)),
            pltpu.SemaphoreType.DMA((NK + 1,)),
            pltpu.SemaphoreType.DMA((len(OUT_CHUNKS),)),
        ],
        compiler_params=pltpu.CompilerParams(vmem_limit_bytes=100 * 1024 * 1024),
    )(A_x, A_wqkv, A_wo, B_w1, B_b1, B_w2, B_b2, gate_w)
```
